```python
import os as _os
_os.environ.setdefault("JAX_PLATFORMS", "cpu")
import jax
import jax.numpy as jnp

def _softmax(x, axis=-1):
    return jax.nn.softmax(x, axis=axis)
def _gelu(x):
    return jax.nn.gelu(x, approximate=True)
def _silu(x):
    return jax.nn.silu(x)
def _sigmoid(x):
    return jax.nn.sigmoid(x)
def _layernorm(x, axis=-1, eps=1e-5):
    m = jnp.mean(x, axis=axis, keepdims=True)
    v = jnp.var(x, axis=axis, keepdims=True)
    return (x - m) / jnp.sqrt(v + eps)
def _scatter_add(tgt, idx, src, axis=0):
    return tgt.at[idx].add(src)
def _segment_sum(src, seg, n):
    return jax.ops.segment_sum(src, seg, n)
class _Rng:
    def __init__(self, key):
        self._k = key
    def _next(self):
        self._k, sub = jax.random.split(self._k)
        return sub
    def normal(self, shape):
        return jax.random.normal(self._next(), shape, dtype=jnp.bfloat16)
    def randint(self, lo, hi, shape):
        return jax.random.randint(self._next(), shape, lo, hi, dtype=jnp.int32)
    def uniform(self, shape, lo=0.0, hi=1.0):
        return jax.random.uniform(self._next(), shape, jnp.bfloat16, lo, hi)
    def permutation(self, n):
        return jax.random.permutation(self._next(), n)


kernel_name = 'gated_mix__sliding_block__sliding_local_dilated__prompt'

def setup_inputs():
    _rng = _Rng(jax.random.key(int.from_bytes(__import__("os").urandom(4), "little")))
    _w = (lambda a: (lambda t: t.astype(jnp.bfloat16) if jnp.issubdtype(t.dtype, jnp.floating) else t)(jnp.asarray(a)))
    def _A_setup():
        B, S, D = 1, 2048, 640
        return {
            "x": _w((lambda *s: _rng.normal(s) * 0.05)(B, S, D)),
            "wqkv": _w((lambda *s: _rng.normal(s) * 0.8)(D, 3 * D)),
            "wo": _w((lambda *s: _rng.normal(s) * 0.05)(D, D)),
        }
    _A_in = _A_setup()

    def _B_setup():
        B, S, D = 1, 2048, 640
        return {
            "x": _w((lambda *s: _rng.normal(s) * 0.05)(B, S, D)),
            "wqkv": _w((lambda *s: _rng.normal(s) * 0.8)(D, 3 * D)),
            "wo": _w((lambda *s: _rng.normal(s) * 0.05)(D, D)),
        }
    _B_in = _B_setup()

    return {
        "A_x": _A_in["x"],
        "A_wqkv": _A_in["wqkv"],
        "A_wo": _A_in["wo"],
        "B_x": _B_in["x"],
        "B_wqkv": _B_in["wqkv"],
        "B_wo": _B_in["wo"],
        "gate_w": _w((lambda *s: _rng.normal(s) * 0.05)(640) * 16.0),
    }

def reference(A_x, A_wqkv, A_wo, B_x, B_wqkv, B_wo, gate_w):
    def _A_ref(x, wqkv, wo):
        B, S, D = x.shape
        H = 32; Dh = D // H; W = 256
        qkv = (lambda x, *d: x.transpose(*d))((x @ wqkv).reshape(B, S, 3, H, Dh), 2, 0, 3, 1, 4)
        q, k, v = qkv[0], qkv[1], qkv[2]
        scores = jnp.einsum("bhqd,bhkd->bhqk", q, k) * (Dh ** -0.5)
        idx = jnp.arange(S)
        mask = (idx[:, None] - idx[None, :] >= 0) & (idx[:, None] - idx[None, :] < W)
        scores = jnp.where(mask[None, None], scores, -1e9)
        p = _softmax(scores, axis=-1)
        o = jnp.einsum("bhqk,bhkd->bhqd", p, v)
        return (lambda x, *d: x.transpose(*d))(o, 0, 2, 1, 3).reshape(B, S, D) @ wo

    def _B_ref(x, wqkv, wo):
        B, S, D = x.shape
        H = 32; Dh = D // H
        W, dil = 8, 2
        qkv = (lambda x, *d: x.transpose(*d))((x @ wqkv).reshape(B, S, 3, H, Dh), 2, 0, 3, 1, 4)
        q, k, v = qkv[0], qkv[1], qkv[2]
        scale = Dh ** -0.5
        pos = jnp.arange(S)
        off = jnp.arange(W) * dil
        idx = pos[:, None] - off[None, :]
        mask = idx >= 0
        idx_c = jnp.where(mask, idx, 0).reshape(-1)
        kg = k[:, :, idx_c, :].reshape(B, H, S, W, Dh)
        vg = v[:, :, idx_c, :].reshape(B, H, S, W, Dh)
        logits = jnp.einsum("bhsd,bhswd->bhsw", q, kg) * scale
        logits = jnp.where(mask[None, None, :, :], logits, -1e9)
        attn = _softmax(logits, axis=-1)
        o = jnp.einsum("bhsw,bhswd->bhsd", attn, vg)
        return (lambda x, *d: x.transpose(*d))(o, 0, 2, 1, 3).reshape(B, S, D) @ wo

    x = A_x
    g = _sigmoid((x * gate_w).sum(-1, keepdims=True))
    a = _A_ref(x, A_wqkv, A_wo)
    b = _B_ref(x, B_wqkv, B_wo)
    return g * a + (1 - g) * b
```

```python
import functools
import jax
import jax.numpy as jnp
import jax.experimental.pallas as pl
import jax.experimental.pallas.tpu as pltpu

S = 2048
D = 640
H = 32
DH = 20
W_B = 8
DIL = 2
TQ = 256
NSTEP = S // TQ
SUB = 128
NSB = TQ // SUB
PAD = 256
LOG2E = 1.4426950408889634
QSCALE = (DH ** -0.5) * LOG2E
NEG = -1e9
HIST = 16
NG = 8
GH = 4
G_OFF = (0, 64, 128, 192, 320, 384, 448, 512)
BCH = 16


def _bias_lane(g):
    lo = 80 * g - G_OFF[g]
    return lo + 80 if lo + 80 < 128 else 0


def _vwin(h):
    base = 16 * ((DH * h) // 16)
    o = DH * h - base
    r = o + DH if o + DH < 32 else 0
    return base, o, r


def _kernel(x_ref, wa_ref, woa_ref, wb_ref, wob_ref, gw_ref, o_ref,
            k_scr, vt_scr, q_scr, ot_scr, wtf_scr, wtp_scr, wobp_scr, qb_scr, kb_scr, vb_scr, ob_scr, g_scr):
    step = pl.program_id(0)
    f32, bf16 = jnp.float32, jnp.bfloat16

    @pl.when(step == 0)
    def _prep():
        lane = jax.lax.broadcasted_iota(jnp.int32, (PAD, 128), 1)
        for g in range(NG):
            k_scr[g, TQ:TQ + PAD, :] = jnp.where(lane == _bias_lane(g), NEG, 0.0).astype(bf16)
        vt_scr[:, :, TQ:TQ + PAD] = jnp.zeros((H, 32, PAD), bf16)
        kb_scr[:, TQ:TQ + HIST, :] = jnp.zeros((5, HIST, 128), f32)
        vb_scr[:, TQ:TQ + HIST, :] = jnp.zeros((5, HIST, 128), f32)
        for j in range(5):
            wtf_scr[...] = wb_ref[128 * j:128 * j + 128, :].astype(f32).T
            for p in range(3):
                for d in range(DH):
                    rows = wtf_scr[pl.ds(p * D + d, H, stride=DH), :]
                    wtp_scr[p * D + H * d:p * D + H * d + H, 128 * j:128 * j + 128] = rows.astype(bf16)
        for j in range(5):
            wtf_scr[0:D, :] = wob_ref[:, 128 * j:128 * j + 128].astype(f32)
            for d in range(DH):
                rows = wtf_scr[pl.ds(d, H, stride=DH), :]
                wobp_scr[H * d:H * d + H, 128 * j:128 * j + 128] = rows.astype(bf16)

    k_scr[:, 0:PAD, :] = k_scr[:, TQ:TQ + PAD, :]
    vt_scr[:, :, 0:PAD] = vt_scr[:, :, TQ:TQ + PAD]
    kb_scr[:, 0:HIST, :] = kb_scr[:, TQ:TQ + HIST, :]
    vb_scr[:, 0:HIST, :] = vb_scr[:, TQ:TQ + HIST, :]

    x = x_ref[...]
    row0 = step * TQ

    ka = jnp.dot(x, wa_ref[:, D:2 * D], preferred_element_type=f32)
    qa = jnp.dot(x, wa_ref[:, 0:D], preferred_element_type=f32) * QSCALE
    lane_t = jax.lax.broadcasted_iota(jnp.int32, (TQ, 128), 1)
    for g in range(NG):
        off = G_OFF[g]
        isb = lane_t == _bias_lane(g)
        k_scr[g, PAD:PAD + TQ, :] = jnp.where(isb, 0.0, ka[:, off:off + 128]).astype(bf16)
        q_scr[g] = jnp.where(isb, 1.0, qa[:, off:off + 128]).astype(bf16)
    va = jnp.dot(x, wa_ref[:, 2 * D:3 * D], preferred_element_type=f32)
    vat = va.T
    rid = jax.lax.broadcasted_iota(jnp.int32, (32, TQ), 0)
    for h in range(H):
        base, o, r = _vwin(h)
        win = jnp.where(rid == r, 1.0, vat[base:base + 32, :])
        vt_scr[h, :, PAD:PAD + TQ] = win.astype(bf16)

    qkvb = jax.lax.dot_general(x, wtp_scr[...], (((1,), (1,)), ((), ())), preferred_element_type=f32)
    for c in range(5):
        qb_scr[c] = qkvb[:, 128 * c:128 * c + 128] * QSCALE
        kb_scr[c, HIST:HIST + TQ, :] = qkvb[:, D + 128 * c:D + 128 * c + 128]
        vb_scr[c, HIST:HIST + TQ, :] = qkvb[:, 2 * D + 128 * c:2 * D + 128 * c + 128]

    gate = jax.nn.sigmoid(jnp.sum(x.astype(f32) * gw_ref[...].astype(f32), axis=1, keepdims=True))
    g_scr[...] = jnp.broadcast_to(gate, (TQ, 128))

    kj = jax.lax.broadcasted_iota(jnp.int32, (SUB, SUB), 0)
    qi = jax.lax.broadcasted_iota(jnp.int32, (SUB, SUB), 1)
    old_valid = kj > qi
    lane = jax.lax.broadcasted_iota(jnp.int32, (SUB, 128), 1)

    def qk(idx):
        sb, g = divmod(idx, NG)
        q = q_scr[g, sb * SUB:(sb + 1) * SUB, :].astype(f32)
        kk = k_scr[g, sb * SUB:sb * SUB + 3 * SUB, :]
        res = []
        for j in range(GH):
            lo = DH * (GH * g + j) - G_OFF[g]
            msk = ((lane >= lo) & (lane < lo + DH)) | (lane == _bias_lane(g))
            qm = jnp.where(msk, q, 0.0).astype(bf16)
            st = jax.lax.dot_general(kk, qm, (((1,), (1,)), ((), ())), preferred_element_type=f32)
            s_mrg = jnp.where(old_valid, st[0:SUB], st[2 * SUB:3 * SUB])
            s_mid = st[SUB:2 * SUB]
            m = jnp.max(jnp.maximum(s_mrg, s_mid), axis=0, keepdims=True)
            res.append((s_mrg, s_mid, m))
        return res

    def softmax_pv(idx, res):
        sb, g = divmod(idx, NG)
        for j in range(GH):
            h = GH * g + j
            s_mrg, s_mid, m = res[j]
            p_mrg = jnp.exp2(s_mrg - m)
            p_mid = jnp.exp2(s_mid - m)
            p_old = jnp.where(old_valid, p_mrg, 0.0)
            p_new = jnp.where(old_valid, 0.0, p_mrg)
            pt = jnp.concatenate([p_old, p_mid, p_new], axis=0).astype(bf16)
            vt = vt_scr[h, :, sb * SUB:sb * SUB + 3 * SUB]
            ot = jnp.dot(vt, pt, preferred_element_type=f32)
            base, o, r = _vwin(h)
            inv = 1.0 / ot[r:r + 1, :]
            ot_scr[DH * h:DH * h + DH, sb * SUB:(sb + 1) * SUB] = ot[o:o + DH, :] * inv

    def b_chunk(ci):
        r0 = ci * BCH
        qb = [qb_scr[c, r0:r0 + BCH, :] for c in range(5)]
        logits = []
        for w in range(W_B):
            off = HIST - DIL * w + r0
            acc = qb[0] * kb_scr[0, off:off + BCH, :]
            for c in range(1, 5):
                acc = acc + qb[c] * kb_scr[c, off:off + BCH, :]
            acc = acc + pltpu.roll(acc, 64, 1)
            acc = acc + pltpu.roll(acc, 32, 1)
            if w > 0 and r0 < DIL * (W_B - 1):
                pos = row0 + r0 + jax.lax.broadcasted_iota(jnp.int32, (BCH, 128), 0)
                acc = jnp.where(pos >= DIL * w, acc, NEG)
            logits.append(acc)
        m = functools.reduce(jnp.maximum, logits)
        es = [jnp.exp2(l - m) for l in logits]
        den = functools.reduce(lambda a, b: a + b, es)
        fac = (1.0 - g_scr[r0:r0 + BCH, :]) / den
        for c in range(5):
            acc = None
            for w in range(W_B):
                off = HIST - DIL * w + r0
                term = es[w] * vb_scr[c, off:off + BCH, :]
                acc = term if acc is None else acc + term
            ob_scr[r0:r0 + BCH, 128 * c:128 * c + 128] = (acc * fac).astype(bf16)

    def out_proj(sb):
        rs = slice(sb * SUB, (sb + 1) * SUB)
        gg = g_scr[rs, :]
        oa = ot_scr[:, rs].T
        oa = jnp.concatenate([oa[:, 128 * c:128 * c + 128] * gg for c in range(5)], axis=1).astype(bf16)
        out = jnp.dot(ob_scr[rs, :], wobp_scr[...], preferred_element_type=f32) + jnp.dot(oa, woa_ref[...], preferred_element_type=f32)
        o_ref[rs, :] = out.astype(o_ref.dtype)

    nidx = NSB * NG
    nch = TQ // BCH
    nxt = qk(0)
    for idx in range(nidx):
        cur = nxt
        if idx + 1 < nidx:
            nxt = qk(idx + 1)
        else:
            out_proj(0)
        softmax_pv(idx, cur)
        for ci in range(idx * nch // nidx, (idx + 1) * nch // nidx):
            b_chunk(ci)
    out_proj(1)


@jax.jit
def pallas_gated_mix__sliding_block__sliding_local_dilated__prompt_kernel(A_x, A_wqkv, A_wo, B_x, B_wqkv, B_wo, gate_w):
    x = A_x.reshape(S, D)
    gw = gate_w.reshape(1, D)
    f32, bf16 = jnp.float32, jnp.bfloat16
    full = lambda shape: pl.BlockSpec(shape, lambda i: (0,) * len(shape))
    out = pl.pallas_call(
        _kernel,
        grid=(NSTEP,),
        in_specs=[
            pl.BlockSpec((TQ, D), lambda i: (i, 0)),
            full((D, 3 * D)), full((D, D)), full((D, 3 * D)), full((D, D)), full((1, D)),
        ],
        out_specs=pl.BlockSpec((TQ, D), lambda i: (i, 0)),
        out_shape=jax.ShapeDtypeStruct((S, D), bf16),
        scratch_shapes=[
            pltpu.VMEM((NG, PAD + TQ, 128), bf16),
            pltpu.VMEM((H, 32, PAD + TQ), bf16),
            pltpu.VMEM((NG, TQ, 128), bf16),
            pltpu.VMEM((D, TQ), f32),
            pltpu.VMEM((3 * D, 128), f32),
            pltpu.VMEM((3 * D, D), bf16),
            pltpu.VMEM((D, D), bf16),
            pltpu.VMEM((5, TQ, 128), f32),
            pltpu.VMEM((5, HIST + TQ, 128), f32),
            pltpu.VMEM((5, HIST + TQ, 128), f32),
            pltpu.VMEM((TQ, D), bf16),
            pltpu.VMEM((TQ, 128), f32),
        ],
        compiler_params=pltpu.CompilerParams(
            dimension_semantics=("arbitrary",),
            vmem_limit_bytes=100 * 1024 * 1024,
        ),
    )(x, A_wqkv, A_wo, B_wqkv, B_wo, gw)
    return out.reshape(1, S, D)
```

```python
import functools
import jax
import jax.numpy as jnp
import jax.experimental.pallas as pl
import jax.experimental.pallas.tpu as pltpu

S = 2048
D = 640
H = 32
DH = 20
W_B = 8
DIL = 2
TQ = 256
NSTEP = S // TQ
SUB = 128
NSB = TQ // SUB
PAD = 256
LOG2E = 1.4426950408889634
QSCALE = (DH ** -0.5) * LOG2E
NEG = -1e9
HIST = 16
NG = 8
GH = 4
QB = 32
NU = PAD // QB + 1
G_OFF = (0, 64, 128, 192, 320, 384, 448, 512)
BCH = 8
BCHAIN = 2
BCHAIN0 = 4

f32, bf16, u32 = jnp.float32, jnp.bfloat16, jnp.uint32
NT = (((1,), (1,)), ((), ()))


def _vwin(h):
    base = 16 * ((DH * h) // 16)
    o = DH * h - base
    r = o + DH if o + DH < 32 else 0
    return base, o, r


def _pack16(v):
    n = v.shape[0] // 16
    lo = jnp.concatenate([v[16 * i:16 * i + 8] for i in range(n)], axis=0)
    hi = jnp.concatenate([v[16 * i + 8:16 * i + 16] for i in range(n)], axis=0)
    return pltpu.pack_elementwise([lo, hi], packed_dtype=bf16).astype(u32)


def _bf(v):
    return pltpu.bitcast(v, bf16)


def _kernel(x_hbm, wa_hbm, woa_hbm, wb_hbm, wob_hbm, gw_hbm, o_ref,
            x_scr, wa_ref, woa_ref, wb_ref, wob_ref, gw_ref, x_sem, w_sem,
            k_scr, vt_scr, q_scr, ot_scr, wtf_scr, wtp_scr, wobp_scr, qb_scr, kb_scr, vb_scr, ob_scr, g_scr, acc_scr):
    step = pl.program_id(0)

    def x_copy(i):
        return pltpu.make_async_copy(x_hbm.at[i], x_scr.at[i], x_sem.at[i])

    def wa_copy(p):
        return pltpu.make_async_copy(wa_hbm.at[:, p * D:(p + 1) * D], wa_ref.at[:, p * D:(p + 1) * D], w_sem.at[p])

    def wb_copy(j):
        return pltpu.make_async_copy(wb_hbm.at[128 * j:128 * j + 128, :], wb_ref.at[128 * j:128 * j + 128, :],
                                     w_sem.at[3 + j])

    woa_copy = pltpu.make_async_copy(woa_hbm, woa_ref, w_sem.at[8])
    wob_copy = pltpu.make_async_copy(wob_hbm, wob_ref, w_sem.at[9])
    gw_copy = pltpu.make_async_copy(gw_hbm, gw_ref, w_sem.at[10])

    def perm_rows(r0):
        ev = wtf_scr[pl.ds(r0, H // 2, stride=2 * DH), :]
        od = wtf_scr[pl.ds(r0 + DH, H // 2, stride=2 * DH), :]
        return pltpu.pack_elementwise([ev, od], packed_dtype=bf16).astype(u32)

    def prep_wb(j):
        wb_copy(j).wait()
        wtf_scr[...] = wb_ref[128 * j:128 * j + 128, :].astype(f32).T
        for p in range(3):
            for d in range(DH):
                r = (p * D + H * d) // 2
                wtp_scr[r:r + H // 2, 128 * j:128 * j + 128] = perm_rows(p * D + d)

    def prep_wob():
        wob_copy.wait()
        for j in range(5):
            wtf_scr[0:D, :] = wob_ref[:, 128 * j:128 * j + 128].astype(f32)
            for d in range(DH):
                r = H * d // 2
                wobp_scr[r:r + H // 2, 128 * j:128 * j + 128] = perm_rows(d)

    def body(first):
        if first:
            x_copy(0).start()
            wa_copy(2).start()
            gw_copy.start()
            wa_copy(1).start()
            wa_copy(0).start()
            for j in range(5):
                wb_copy(j).start()
            wob_copy.start()
            woa_copy.start()
            for i in range(1, NSTEP):
                x_copy(i).start()
            kb_scr[:, 0:HIST, :] = jnp.zeros((5, HIST, 128), f32)
            vb_scr[:, 0:HIST, :] = jnp.zeros((5, HIST, 128), f32)
            x_copy(0).wait()
            gw_copy.wait()
            x_ref = x_scr.at[0]
        else:
            x_copy(step).wait()
            x_ref = x_scr.at[step]
            k_scr[:, 0:PAD // 2, :] = k_scr[:, TQ // 2:(TQ + PAD) // 2, :]
            vt_scr[:, :, 0:PAD] = vt_scr[:, :, TQ:TQ + PAD]
            kb_scr[:, 0:HIST, :] = kb_scr[:, TQ:TQ + HIST, :]
            vb_scr[:, 0:HIST, :] = vb_scr[:, TQ:TQ + HIST, :]

        x = x_ref[...]
        never = jax.lax.broadcasted_iota(jnp.int32, (BCH, 128), 0) + step < 0

        xf = x.astype(f32)
        gw = gw_ref[...].astype(f32)
        gate = jax.nn.sigmoid(jnp.sum(xf * gw, axis=1, keepdims=True))
        g_scr[...] = jnp.broadcast_to(gate, (TQ, 128))
        xp = _bf(_pack16(xf))
        xu = pltpu.bitcast(x, u32)
        x_ev = pltpu.unpack_elementwise(xu, index=0, packed_dtype=bf16, unpacked_dtype=f32)
        x_od = pltpu.unpack_elementwise(xu, index=1, packed_dtype=bf16, unpacked_dtype=f32)
        xe = jnp.concatenate([t[8 * i:8 * i + 8] for i in range(TQ // 16) for t in (x_ev, x_od)], axis=0).astype(bf16)

        def proj_b(sb):
            rs = slice(sb * SUB, (sb + 1) * SUB)
            hs = slice(HIST + sb * SUB, HIST + (sb + 1) * SUB)
            qkvb = jax.lax.dot_general(x[rs], _bf(wtp_scr[...]), NT, preferred_element_type=f32)
            for c in range(5):
                qb_scr[c, rs, :] = qkvb[:, 128 * c:128 * c + 128] * QSCALE
                kb_scr[c, hs, :] = qkvb[:, D + 128 * c:D + 128 * c + 128]
                vb_scr[c, hs, :] = qkvb[:, 2 * D + 128 * c:2 * D + 128 * c + 128]

        def b_chunk(ci, dep):
            r0 = ci * BCH
            qb = [qb_scr[c, r0:r0 + BCH, :] for c in range(5)]
            if dep is not None:
                qb = [jnp.where(never, dep, q) for q in qb]
            logits = []
            for w in range(W_B):
                off = HIST - DIL * w + r0
                acc = qb[0] * kb_scr[0, off:off + BCH, :]
                for c in range(1, 5):
                    acc = acc + qb[c] * kb_scr[c, off:off + BCH, :]
                acc = acc + pltpu.roll(acc, 64, 1)
                acc = acc + pltpu.roll(acc, 32, 1)
                if first and r0 < DIL * w:
                    pos = r0 + jax.lax.broadcasted_iota(jnp.int32, (BCH, 128), 0)
                    acc = jnp.where(pos >= DIL * w, acc, NEG)
                logits.append(acc)
            m = functools.reduce(jnp.maximum, logits)
            es = [jnp.exp2(l - m) for l in logits]
            den = functools.reduce(lambda a, b: a + b, es)
            fac = (1.0 - g_scr[r0:r0 + BCH, :]) / den
            for c in range(5):
                acc = None
                for w in range(W_B):
                    off = HIST - DIL * w + r0
                    term = es[w] * vb_scr[c, off:off + BCH, :]
                    acc = term if acc is None else acc + term
                acc = acc * fac
                ob_scr[r0:r0 + BCH, 128 * c:128 * c + 128] = acc.astype(bf16)
            return acc

        def attn_b(chain):
            deps = []
            for ci in range(TQ // BCH):
                deps.append(b_chunk(ci, deps[ci - chain] if chain and ci >= chain else None))

        def emit(sb, v, init, last):
            rs = slice(sb * SUB, (sb + 1) * SUB)
            if not init:
                v = acc_scr[rs, :] + v
            if last:
                o_ref[rs, :] = v.astype(o_ref.dtype)
            else:
                acc_scr[rs, :] = v

        def op_b(sb, init=False, last=False):
            rs = slice(sb * SUB, (sb + 1) * SUB)
            emit(sb, jnp.dot(ob_scr[rs, :], _bf(wobp_scr[...]), preferred_element_type=f32), init, last)

        def op_a(sb, c0, c1, init=False, last=False):
            rs = slice(sb * SUB, (sb + 1) * SUB)
            gg = g_scr[rs, :]
            oa = ot_scr[128 * c0:128 * c1, rs].T
            oa = jnp.concatenate([oa[:, 128 * c:128 * c + 128] * gg for c in range(c1 - c0)], axis=1).astype(bf16)
            emit(sb, jnp.dot(oa, woa_ref[128 * c0:128 * c1, :], preferred_element_type=f32), init, last)

        def proj_v():
            va = jnp.dot(xp, wa_ref[:, 2 * D:3 * D], preferred_element_type=f32)
            vat = va.T
            rid = jax.lax.broadcasted_iota(jnp.int32, (32, TQ), 0)
            for h in range(H):
                base, o, r = _vwin(h)
                win = jnp.where(rid == r, 1.0, vat[base:base + 32, :])
                vt_scr[h, :, PAD:PAD + TQ] = win.astype(bf16)

        def proj_k():
            ka = jnp.dot(xe, wa_ref[:, D:2 * D], preferred_element_type=f32)
            for g in range(NG):
                k_scr[g, PAD // 2:(PAD + TQ) // 2, :] = _pack16(ka[:, G_OFF[g]:G_OFF[g] + 128])

        def proj_q():
            qa = jnp.dot(xe, wa_ref[:, 0:D], preferred_element_type=f32) * QSCALE
            for g in range(NG):
                q_scr[g] = _pack16(qa[:, G_OFF[g]:G_OFF[g] + 128])

        lane = jax.lax.broadcasted_iota(jnp.int32, (QB, 128), 1)
        krow = jax.lax.broadcasted_iota(jnp.int32, (QB, 128), 0)
        old_valid = krow > (lane & (QB - 1))
        lane16 = jax.lax.broadcasted_iota(jnp.int32, (QB // 2, 128), 1)

        def masks(rows):
            slot = jax.lax.broadcasted_iota(jnp.int32, (rows, 128), 1) // QB
            return slot, (slot == 0) | (slot == 2), slot < 2, (slot == 1) | (slot == 2)

        mk16 = masks(QB // 2)
        mk1 = masks(1)

        def butterfly(X, mk):
            slot, m_even, m_01, m_12 = mk

            def sel(m, a, b):
                if a is None and b is None:
                    return None
                z = jnp.zeros_like(a if b is None else b)
                return jnp.where(m, z if a is None else a, z if b is None else b)

            live = [t for t in range(GH) if X[t] is not None]
            if len(live) == 1:
                t = live[0]
                return [sel(slot == (j + t) % GH, X[t], None) for j in range(GH)]
            a0 = sel(m_even, X[0], X[1])
            a1 = sel(m_even, X[1], X[0])
            b0 = sel(m_even, X[2], X[3])
            b1 = sel(m_even, X[3], X[2])
            return [sel(m_01, a0, b0), sel(m_12, a1, b1), sel(m_01, b0, a0), sel(m_12, b1, a1)]

        st8 = {}

        def segs_of(idx):
            sb = idx // NG
            return tuple(range(2 - sb, 3)) if first else (0, 1, 2)

        def qweights(idx, t):
            sb, g = divmod(idx, NG)
            r0 = (sb * SUB + QB * t) // 2
            q = q_scr[g, r0:r0 + QB // 2, :]
            parts = []
            for s in range(GH):
                j = (s - t) % GH
                lo = DH * (GH * g + j) - G_OFF[g]
                parts.append(jnp.where((lane16 >= lo) & (lane16 < lo + DH), q, jnp.zeros_like(q)))
            return _bf(jnp.concatenate(parts, axis=0))

        def seg_range(t, seg):
            return max(4 * seg - t, 0), min(4 * seg + 4 - t, NU)

        def soft(idx, t, seg, chunks):
            S_ = st8.setdefault(idx, {'P': [dict() for _ in range(GH)], 'm': {}, 'o': {}})
            u0, u1 = seg_range(t, seg)
            ss = {}
            for u in range(u0, u1):
                s = chunks[u]
                if u == 0:
                    s = jnp.where(old_valid, s, NEG)
                if u == NU - 1:
                    s = jnp.where(old_valid, NEG, s)
                ss[u] = s
            mx = functools.reduce(jnp.maximum,
                                  [ss[u][8 * i:8 * i + 8] for u in range(u0, u1) for i in range(QB // 8)])
            m = jnp.max(mx, axis=0, keepdims=True)
            S_['m'][(t, seg)] = m
            for u in range(u0, u1):
                S_['P'][t][u] = _pack16(jnp.exp2(ss[u] - m))

        def qk(idx):
            sb, g = divmod(idx, NG)
            segs = segs_of(idx)
            chunks = []
            for t in range(GH):
                u0 = seg_range(t, segs[0])[0]
                r0 = (sb * SUB + QB * t) // 2
                kk = _bf(k_scr[g, r0 + u0 * QB // 2:r0 + NU * QB // 2, :])
                st = jax.lax.dot_general(kk, qweights(idx, t), NT, preferred_element_type=f32)
                chunks.append({u: st[QB * (u - u0):QB * (u - u0) + QB] for u in range(u0, NU)})
            for seg in segs:
                for t in ((3, 2, 1, 0) if seg < 2 else (0, 1, 2, 3)):
                    soft(idx, t, seg, chunks[t])

        def pv(idx):
            sb, g = divmod(idx, NG)
            segs = segs_of(idx)
            S_ = st8.pop(idx)
            for seg in segs:
                outs = [[] for _ in range(GH)]
                for c in range(4 * seg, 4 * seg + 4):
                    X = [S_['P'][t].get(c - t) for t in range(GH)]
                    for j, v in enumerate(butterfly(X, mk16)):
                        outs[j].append(v)
                for j in range(GH):
                    h = GH * g + j
                    pt = _bf(jnp.concatenate(outs[j], axis=0))
                    vt = vt_scr[h, :, (sb + seg) * SUB:(sb + seg + 1) * SUB]
                    S_['o'][(j, seg)] = jnp.dot(vt, pt, preferred_element_type=f32)
            al = {}
            if len(segs) > 1:
                mf = [functools.reduce(jnp.maximum, [S_['m'][(t, seg)] for seg in segs]) for t in range(GH)]
                for seg in segs:
                    al[seg] = butterfly([jnp.exp2(S_['m'][(t, seg)] - mf[t]) for t in range(GH)], mk1)
            for j in range(GH):
                h = GH * g + j
                if len(segs) > 1:
                    ot = functools.reduce(lambda a, b: a + b, [S_['o'][(j, seg)] * al[seg][j] for seg in segs])
                else:
                    ot = S_['o'][(j, segs[0])]
                base, o, r = _vwin(h)
                inv = 1.0 / ot[r:r + 1, :]
                on = ot * inv
                if j:
                    on = pltpu.roll(on, 128 - QB * j, 1)
                ot_scr[DH * h:DH * h + DH, sb * SUB:(sb + 1) * SUB] = on[o:o + DH, :]

        nidx = NSB * NG
        if first:
            wa_copy(2).wait()
            proj_v()
            wa_copy(1).wait()
            proj_k()
            wa_copy(0).wait()
            proj_q()
            extra = {0: lambda: prep_wb(0), 3: lambda: prep_wb(1), 6: lambda: prep_wb(2), 9: lambda: prep_wb(3),
                     11: lambda: prep_wb(4), 13: prep_wob}
            for idx in range(nidx + 1):
                if idx in extra:
                    extra[idx]()
                if idx < nidx:
                    qk(idx)
                else:
                    proj_b(0)
                if idx > 0:
                    pv(idx - 1)
            proj_b(1)
            attn_b(BCHAIN0)
            woa_copy.wait()
            op_a(0, 0, 5, init=True)
            op_a(1, 0, 5, init=True)
            op_b(0, last=True)
            op_b(1, last=True)
        else:
            proj_b(0)
            proj_b(1)
            attn_b(BCHAIN)
            proj_v()
            proj_k()
            op_b(0, init=True)
            proj_q()
            op_b(1, init=True)
            for idx in range(nidx + 1):
                if idx < nidx:
                    qk(idx)
                else:
                    op_a(0, 0, 5, last=True)
                if idx > 0:
                    pv(idx - 1)
            op_a(1, 0, 4)
            op_a(1, 4, 5, last=True)

    @pl.when(step == 0)
    def _():
        body(True)

    @pl.when(step > 0)
    def _():
        body(False)


@jax.jit
def pallas_gated_mix__sliding_block__sliding_local_dilated__prompt_kernel(A_x, A_wqkv, A_wo, B_x, B_wqkv, B_wo, gate_w):
    x = A_x.reshape(NSTEP, TQ, D)
    gw = gate_w.reshape(1, D)
    hbm = pl.BlockSpec(memory_space=pl.ANY)
    out = pl.pallas_call(
        _kernel,
        grid=(NSTEP,),
        in_specs=[hbm] * 6,
        out_specs=pl.BlockSpec((TQ, D), lambda i: (i, 0)),
        out_shape=jax.ShapeDtypeStruct((S, D), bf16),
        scratch_shapes=[
            pltpu.VMEM((NSTEP, TQ, D), bf16),
            pltpu.VMEM((D, 3 * D), bf16),
            pltpu.VMEM((D, D), bf16),
            pltpu.VMEM((D, 3 * D), bf16),
            pltpu.VMEM((D, D), bf16),
            pltpu.VMEM((1, D), bf16),
            pltpu.SemaphoreType.DMA((NSTEP,)),
            pltpu.SemaphoreType.DMA((11,)),
            pltpu.VMEM((NG, (PAD + TQ) // 2, 128), u32),
            pltpu.VMEM((H, 32, PAD + TQ), bf16),
            pltpu.VMEM((NG, TQ // 2, 128), u32),
            pltpu.VMEM((D, TQ), f32),
            pltpu.VMEM((3 * D, 128), f32),
            pltpu.VMEM((3 * D // 2, D), u32),
            pltpu.VMEM((D // 2, D), u32),
            pltpu.VMEM((5, TQ, 128), f32),
            pltpu.VMEM((5, HIST + TQ, 128), f32),
            pltpu.VMEM((5, HIST + TQ, 128), f32),
            pltpu.VMEM((TQ, D), bf16),
            pltpu.VMEM((TQ, 128), f32),
            pltpu.VMEM((TQ, D), f32),
        ],
        compiler_params=pltpu.CompilerParams(
            dimension_semantics=("arbitrary",),
            vmem_limit_bytes=100 * 1024 * 1024,
        ),
    )(x, A_wqkv, A_wo, B_wqkv, B_wo, gw)
    return out.reshape(1, S, D)
```

```python
import functools
import jax
import jax.numpy as jnp
import jax.experimental.pallas as pl
import jax.experimental.pallas.tpu as pltpu

S = 2048
D = 640
H = 32
DH = 20
W_B = 8
DIL = 2
TQ = 256
NSTEP = S // TQ
SUB = 128
NSB = TQ // SUB
LAST = NSTEP - 1
PAD = 256
LOG2E = 1.4426950408889634
QSCALE = (DH ** -0.5) * LOG2E
NEG = -1e9
HIST = 16
NG = 8
GH = 4
QB = 32
NU = PAD // QB + 1
G_OFF = (0, 64, 128, 192, 320, 384, 448, 512)
BCH = 8
BCHAIN = 2
BCHAIN0 = 4
S0 = (3, 14)

f32, bf16, u32 = jnp.float32, jnp.bfloat16, jnp.uint32
NT = (((1,), (1,)), ((), ()))


def _vwin(h):
    base = 16 * ((DH * h) // 16)
    o = DH * h - base
    r = o + DH if o + DH < 32 else 0
    return base, o, r


def _pack16(v):
    n = v.shape[0] // 16
    lo = jnp.concatenate([v[16 * i:16 * i + 8] for i in range(n)], axis=0)
    hi = jnp.concatenate([v[16 * i + 8:16 * i + 16] for i in range(n)], axis=0)
    return pltpu.pack_elementwise([lo, hi], packed_dtype=bf16).astype(u32)


def _bf(v):
    return pltpu.bitcast(v, bf16)


def _kernel(x_hbm, wa_hbm, woa_hbm, wb_hbm, wob_hbm, gw_hbm, o_ref,
            x_scr, wa_ref, woa_ref, wb_ref, wob_ref, gw_ref, x_sem, w_sem,
            k_scr, vt_scr, q_scr, ot_scr, wtf_scr, wtp_scr, wobp_scr, qb_scr, kb_scr, vb_scr, ob_scr, g_scr, acc_scr):
    step = pl.program_id(0)

    def x_copy(i):
        return pltpu.make_async_copy(x_hbm.at[i], x_scr.at[i], x_sem.at[i])

    def wa_copy(p):
        return pltpu.make_async_copy(wa_hbm.at[:, p * D:(p + 1) * D], wa_ref.at[:, p * D:(p + 1) * D], w_sem.at[p])

    def wb_copy(p):
        return pltpu.make_async_copy(wb_hbm.at[:, p * D:(p + 1) * D], wb_ref.at[:, p * D:(p + 1) * D], w_sem.at[3 + p])

    woa_copy = pltpu.make_async_copy(woa_hbm, woa_ref, w_sem.at[6])
    wob_copy = pltpu.make_async_copy(wob_hbm, wob_ref, w_sem.at[7])
    gw_copy = pltpu.make_async_copy(gw_hbm, gw_ref, w_sem.at[8])

    def prep_wb(p):
        for j in range(5):
            jj = j + 5 * (p % 2)
            wtf_scr[jj] = wb_ref[128 * j:128 * j + 128, p * D:(p + 1) * D].astype(f32).T
            for d in range(DH):
                r = (p * D + H * d) // 2
                wtp_scr[r:r + H // 2, 128 * j:128 * j + 128] = _pack16(wtf_scr[jj, pl.ds(d, H, stride=DH), :])

    def prep_wob():
        for j in range(5):
            wtf_scr[j] = wob_ref[:, 128 * j:128 * j + 128].astype(f32)
            for d in range(DH):
                r = H * d // 2
                wobp_scr[r:r + H // 2, 128 * j:128 * j + 128] = _pack16(wtf_scr[j, pl.ds(d, H, stride=DH), :])

    def body(first):
        if first:
            x_copy(0).start()
            wa_copy(2).start()
            gw_copy.start()
            wa_copy(1).start()
            wa_copy(0).start()
            for p in range(3):
                wb_copy(p).start()
            wob_copy.start()
            woa_copy.start()
            x_copy(1).start()
            kb_scr[:, 0:HIST, :] = jnp.zeros((5, HIST, 128), f32)
            vb_scr[:, 0:HIST, :] = jnp.zeros((5, HIST, 128), f32)
            x_copy(0).wait()
            gw_copy.wait()
            x_ref = x_scr.at[0]
        else:
            x_copy(step).wait()

            @pl.when(step < LAST)
            def _():
                x_copy(step + 1).start()

            x_ref = x_scr.at[step]
            k_scr[:, 0:PAD // 2, :] = k_scr[:, TQ // 2:(TQ + PAD) // 2, :]
            vt_scr[:, :, 0:PAD] = vt_scr[:, :, TQ:TQ + PAD]
            kb_scr[:, 0:HIST, :] = kb_scr[:, TQ:TQ + HIST, :]
            vb_scr[:, 0:HIST, :] = vb_scr[:, TQ:TQ + HIST, :]

        x = x_ref[...]
        never = jax.lax.broadcasted_iota(jnp.int32, (BCH, 128), 0) + step < 0

        xf = x.astype(f32)
        gw = gw_ref[...].astype(f32)
        gate = jax.nn.sigmoid(jnp.sum(xf * gw, axis=1, keepdims=True))
        g_scr[...] = jnp.broadcast_to(gate, (TQ, 128))
        xp = _bf(_pack16(xf))
        xu = pltpu.bitcast(x, u32)
        x_ev = pltpu.unpack_elementwise(xu, index=0, packed_dtype=bf16, unpacked_dtype=f32)
        x_od = pltpu.unpack_elementwise(xu, index=1, packed_dtype=bf16, unpacked_dtype=f32)
        xe = jnp.concatenate([t[8 * i:8 * i + 8] for i in range(TQ // 16) for t in (x_ev, x_od)], axis=0).astype(bf16)

        def proj_b(sb):
            rs = slice(sb * SUB, (sb + 1) * SUB)
            hs = slice(HIST + sb * SUB, HIST + (sb + 1) * SUB)
            qkvb = jax.lax.dot_general(x[rs], _bf(wtp_scr[...]), NT, preferred_element_type=f32)
            for c in range(5):
                qb_scr[c, rs, :] = qkvb[:, 128 * c:128 * c + 128] * QSCALE
                kb_scr[c, hs, :] = qkvb[:, D + 128 * c:D + 128 * c + 128]
                vb_scr[c, hs, :] = qkvb[:, 2 * D + 128 * c:2 * D + 128 * c + 128]

        def proj_b_part(p, r0=0, r1=TQ):
            res = jax.lax.dot_general(x[r0:r1], _bf(wtp_scr[p * D // 2:(p + 1) * D // 2, :]), NT,
                                      preferred_element_type=f32)
            for c in range(5):
                v = res[:, 128 * c:128 * c + 128]
                if p == 0:
                    qb_scr[c, r0:r1, :] = v * QSCALE
                elif p == 1:
                    kb_scr[c, HIST + r0:HIST + r1, :] = v
                else:
                    vb_scr[c, HIST + r0:HIST + r1, :] = v

        def b_chunk(ci, dep):
            r0 = ci * BCH
            qb = [qb_scr[c, r0:r0 + BCH, :] for c in range(5)]
            if dep is not None:
                qb = [jnp.where(never, dep, q) for q in qb]
            logits = []
            for w in range(W_B):
                off = HIST - DIL * w + r0
                acc = qb[0] * kb_scr[0, off:off + BCH, :]
                for c in range(1, 5):
                    acc = acc + qb[c] * kb_scr[c, off:off + BCH, :]
                acc = acc + pltpu.roll(acc, 64, 1)
                acc = acc + pltpu.roll(acc, 32, 1)
                if first and r0 < DIL * w:
                    pos = r0 + jax.lax.broadcasted_iota(jnp.int32, (BCH, 128), 0)
                    acc = jnp.where(pos >= DIL * w, acc, NEG)
                logits.append(acc)
            m = functools.reduce(jnp.maximum, logits)
            es = [jnp.exp2(l - m) for l in logits]
            den = functools.reduce(lambda a, b: a + b, es)
            fac = (1.0 - g_scr[r0:r0 + BCH, :]) / den
            for c in range(5):
                acc = None
                for w in range(W_B):
                    off = HIST - DIL * w + r0
                    term = es[w] * vb_scr[c, off:off + BCH, :]
                    acc = term if acc is None else acc + term
                acc = acc * fac
                ob_scr[r0:r0 + BCH, 128 * c:128 * c + 128] = acc.astype(bf16)
            return acc

        def attn_b(chain):
            deps = []
            for ci in range(TQ // BCH):
                deps.append(b_chunk(ci, deps[ci - chain] if chain and ci >= chain else None))

        def emit(sb, v, init, last):
            rs = slice(sb * SUB, (sb + 1) * SUB)
            if not init:
                v = acc_scr[rs, :] + v
            if last:
                o_ref[rs, :] = v.astype(o_ref.dtype)
            else:
                acc_scr[rs, :] = v

        def op_b(sb, init=False, last=False):
            rs = slice(sb * SUB, (sb + 1) * SUB)
            emit(sb, jnp.dot(ob_scr[rs, :], _bf(wobp_scr[...]), preferred_element_type=f32), init, last)

        def op_a(sb, c0, c1, init=False, last=False):
            rs = slice(sb * SUB, (sb + 1) * SUB)
            gg = g_scr[rs, :]
            oa = ot_scr[128 * c0:128 * c1, rs].T
            oa = jnp.concatenate([oa[:, 128 * c:128 * c + 128] * gg for c in range(c1 - c0)], axis=1).astype(bf16)
            emit(sb, jnp.dot(oa, woa_ref[128 * c0:128 * c1, :], preferred_element_type=f32), init, last)

        def dot_a(p):
            return jnp.dot(xp if p == 2 else xe, wa_ref[:, p * D:(p + 1) * D], preferred_element_type=f32)

        def post_v(va):
            vat = va.T
            rid = jax.lax.broadcasted_iota(jnp.int32, (32, TQ), 0)
            for h in range(H):
                base, o, r = _vwin(h)
                win = jnp.where(rid == r, 1.0, vat[base:base + 32, :])
                vt_scr[h, :, PAD:PAD + TQ] = win.astype(bf16)

        def post_k(ka):
            for g in range(NG):
                k_scr[g, PAD // 2:(PAD + TQ) // 2, :] = _pack16(ka[:, G_OFF[g]:G_OFF[g] + 128])

        def post_q(qa):
            qa = qa * QSCALE
            for g in range(NG):
                q_scr[g] = _pack16(qa[:, G_OFF[g]:G_OFF[g] + 128])

        lane = jax.lax.broadcasted_iota(jnp.int32, (QB, 128), 1)
        krow = jax.lax.broadcasted_iota(jnp.int32, (QB, 128), 0)
        old_valid = krow > (lane & (QB - 1))
        lane16 = jax.lax.broadcasted_iota(jnp.int32, (QB // 2, 128), 1)

        def masks(rows):
            slot = jax.lax.broadcasted_iota(jnp.int32, (rows, 128), 1) // QB
            return slot, (slot == 0) | (slot == 2), slot < 2, (slot == 1) | (slot == 2)

        mk16 = masks(QB // 2)
        mk1 = masks(1)

        def butterfly(X, mk):
            slot, m_even, m_01, m_12 = mk

            def sel(m, a, b):
                if a is None and b is None:
                    return None
                z = jnp.zeros_like(a if b is None else b)
                return jnp.where(m, z if a is None else a, z if b is None else b)

            live = [t for t in range(GH) if X[t] is not None]
            if len(live) == 1:
                t = live[0]
                return [sel(slot == (j + t) % GH, X[t], None) for j in range(GH)]
            a0 = sel(m_even, X[0], X[1])
            a1 = sel(m_even, X[1], X[0])
            b0 = sel(m_even, X[2], X[3])
            b1 = sel(m_even, X[3], X[2])
            return [sel(m_01, a0, b0), sel(m_12, a1, b1), sel(m_01, b0, a0), sel(m_12, b1, a1)]

        st8 = {}

        def segs_of(idx):
            sb = idx // NG
            return tuple(range(2 - sb, 3)) if first else (0, 1, 2)

        def qweights(idx, t):
            sb, g = divmod(idx, NG)
            r0 = (sb * SUB + QB * t) // 2
            q = q_scr[g, r0:r0 + QB // 2, :]
            parts = []
            for s in range(GH):
                j = (s - t) % GH
                lo = DH * (GH * g + j) - G_OFF[g]
                parts.append(jnp.where((lane16 >= lo) & (lane16 < lo + DH), q, jnp.zeros_like(q)))
            return _bf(jnp.concatenate(parts, axis=0))

        def seg_range(t, seg):
            return max(4 * seg - t, 0), min(4 * seg + 4 - t, NU)

        def soft(idx, t, seg, chunks):
            S_ = st8.setdefault(idx, {'P': [dict() for _ in range(GH)], 'm': {}, 'o': {}})
            u0, u1 = seg_range(t, seg)
            ss = {}
            for u in range(u0, u1):
                s = chunks[u]
                if u == 0:
                    s = jnp.where(old_valid, s, NEG)
                if u == NU - 1:
                    s = jnp.where(old_valid, NEG, s)
                ss[u] = s
            mx = functools.reduce(jnp.maximum,
                                  [ss[u][8 * i:8 * i + 8] for u in range(u0, u1) for i in range(QB // 8)])
            m = jnp.max(mx, axis=0, keepdims=True)
            S_['m'][(t, seg)] = m
            for u in range(u0, u1):
                S_['P'][t][u] = _pack16(jnp.exp2(ss[u] - m))

        def qk(idx):
            sb, g = divmod(idx, NG)
            segs = segs_of(idx)
            chunks = []
            for t in range(GH):
                u0 = seg_range(t, segs[0])[0]
                r0 = (sb * SUB + QB * t) // 2
                kk = _bf(k_scr[g, r0 + u0 * QB // 2:r0 + NU * QB // 2, :])
                st = jax.lax.dot_general(kk, qweights(idx, t), NT, preferred_element_type=f32)
                chunks.append({u: st[QB * (u - u0):QB * (u - u0) + QB] for u in range(u0, NU)})
            for seg in segs:
                for t in ((3, 2, 1, 0) if seg < 2 else (0, 1, 2, 3)):
                    soft(idx, t, seg, chunks[t])

        def pv(idx):
            sb, g = divmod(idx, NG)
            segs = segs_of(idx)
            S_ = st8.pop(idx)
            for seg in segs:
                outs = [[] for _ in range(GH)]
                for c in range(4 * seg, 4 * seg + 4):
                    X = [S_['P'][t].get(c - t) for t in range(GH)]
                    for j, v in enumerate(butterfly(X, mk16)):
                        outs[j].append(v)
                for j in range(GH):
                    h = GH * g + j
                    pt = _bf(jnp.concatenate(outs[j], axis=0))
                    vt = vt_scr[h, :, (sb + seg) * SUB:(sb + seg + 1) * SUB]
                    S_['o'][(j, seg)] = jnp.dot(vt, pt, preferred_element_type=f32)
            al = {}
            if len(segs) > 1:
                mf = [functools.reduce(jnp.maximum, [S_['m'][(t, seg)] for seg in segs]) for t in range(GH)]
                for seg in segs:
                    al[seg] = butterfly([jnp.exp2(S_['m'][(t, seg)] - mf[t]) for t in range(GH)], mk1)
            for j in range(GH):
                h = GH * g + j
                if len(segs) > 1:
                    ot = functools.reduce(lambda a, b: a + b, [S_['o'][(j, seg)] * al[seg][j] for seg in segs])
                else:
                    ot = S_['o'][(j, segs[0])]
                base, o, r = _vwin(h)
                inv = 1.0 / ot[r:r + 1, :]
                on = ot * inv
                if j:
                    on = pltpu.roll(on, 128 - QB * j, 1)
                ot_scr[DH * h:DH * h + DH, sb * SUB:(sb + 1) * SUB] = on[o:o + DH, :]

        nidx = NSB * NG

        def attn(i0, i1):
            for idx in range(i0, i1):
                if idx < nidx:
                    qk(idx)
                if idx > 0:
                    pv(idx - 1)

        if first:
            wa_copy(2).wait()
            va = dot_a(2)
            wa_copy(1).wait()
            ka = dot_a(1)
            post_v(va)
            wa_copy(0).wait()
            qa = dot_a(0)
            post_k(ka)
            post_q(qa)
            attn(0, S0[0])
            wb_copy(0).wait()
            prep_wb(0)
            attn(S0[0], S0[1])
            wb_copy(1).wait()
            wb_copy(2).wait()
            prep_wb(1)
            prep_wb(2)
            attn(S0[1], nidx)
            proj_b_part(0)
            attn(nidx, nidx + 1)
            proj_b_part(1)
            wob_copy.wait()
            woa_copy.wait()
            proj_b_part(2, 0, SUB)
            proj_b_part(2, SUB, TQ)
            prep_wob()
            attn_b(BCHAIN0)
            op_a(0, 0, 5, init=True)
            op_a(1, 0, 5, init=True)
            op_b(0, last=True)
            op_b(1, last=True)
        else:
            proj_b(0)
            proj_b(1)
            attn_b(BCHAIN)
            post_v(dot_a(2))
            post_k(dot_a(1))
            op_b(0, init=True)
            post_q(dot_a(0))
            op_b(1, init=True)
            attn(0, nidx)
            op_a(0, 0, 5, last=True)
            attn(nidx, nidx + 1)
            op_a(1, 0, 4)
            op_a(1, 4, 5, last=True)

    @pl.when(step == 0)
    def _():
        body(True)

    @pl.when(step > 0)
    def _():
        body(False)


@jax.jit
def pallas_gated_mix__sliding_block__sliding_local_dilated__prompt_kernel(A_x, A_wqkv, A_wo, B_x, B_wqkv, B_wo, gate_w):
    x = A_x.reshape(NSTEP, TQ, D)
    gw = gate_w.reshape(1, D)
    hbm = pl.BlockSpec(memory_space=pl.ANY)
    out = pl.pallas_call(
        _kernel,
        grid=(NSTEP,),
        in_specs=[hbm] * 6,
        out_specs=pl.BlockSpec((TQ, D), lambda i: (i, 0)),
        out_shape=jax.ShapeDtypeStruct((S, D), bf16),
        scratch_shapes=[
            pltpu.VMEM((NSTEP, TQ, D), bf16),
            pltpu.VMEM((D, 3 * D), bf16),
            pltpu.VMEM((D, D), bf16),
            pltpu.VMEM((D, 3 * D), bf16),
            pltpu.VMEM((D, D), bf16),
            pltpu.VMEM((1, D), bf16),
            pltpu.SemaphoreType.DMA((NSTEP,)),
            pltpu.SemaphoreType.DMA((9,)),
            pltpu.VMEM((NG, (PAD + TQ) // 2, 128), u32),
            pltpu.VMEM((H, 32, PAD + TQ), bf16),
            pltpu.VMEM((NG, TQ // 2, 128), u32),
            pltpu.VMEM((D, TQ), f32),
            pltpu.VMEM((10, D, 128), f32),
            pltpu.VMEM((3 * D // 2, D), u32),
            pltpu.VMEM((D // 2, D), u32),
            pltpu.VMEM((5, TQ, 128), f32),
            pltpu.VMEM((5, HIST + TQ, 128), f32),
            pltpu.VMEM((5, HIST + TQ, 128), f32),
            pltpu.VMEM((TQ, D), bf16),
            pltpu.VMEM((TQ, 128), f32),
            pltpu.VMEM((TQ, D), f32),
        ],
        compiler_params=pltpu.CompilerParams(
            dimension_semantics=("arbitrary",),
            vmem_limit_bytes=100 * 1024 * 1024,
        ),
    )(x, A_wqkv, A_wo, B_wqkv, B_wo, gw)
    return out.reshape(1, S, D)
```

```python
import functools
import jax
import jax.numpy as jnp
import jax.experimental.pallas as pl
import jax.experimental.pallas.tpu as pltpu

S = 2048
D = 640
H = 32
DH = 20
W_B = 8
DIL = 2
TQ = 256
NSTEP = S // TQ
SUB = 128
NSB = TQ // SUB
LAST = NSTEP - 1
PAD = 256
LOG2E = 1.4426950408889634
QSCALE = (DH ** -0.5) * LOG2E
NEG = -1e9
HIST = 16
NG = 8
GH = 4
QB = 32
NU = PAD // QB + 1
G_OFF = (0, 64, 128, 192, 320, 384, 448, 512)
BCH = 8
BCHAIN = 2
BCHAIN0 = 4
WA_CH = ((1408, 1920), (896, 1408), (384, 896), (0, 384))

f32, bf16, u32 = jnp.float32, jnp.bfloat16, jnp.uint32
NT = (((1,), (1,)), ((), ()))


def _vwin(h):
    base = 16 * ((DH * h) // 16)
    o = DH * h - base
    r = o + DH if o + DH < 32 else 0
    return base, o, r


def _pack16(v):
    n = v.shape[0] // 16
    lo = jnp.concatenate([v[16 * i:16 * i + 8] for i in range(n)], axis=0)
    hi = jnp.concatenate([v[16 * i + 8:16 * i + 16] for i in range(n)], axis=0)
    return pltpu.pack_elementwise([lo, hi], packed_dtype=bf16).astype(u32)


def _bf(v):
    return pltpu.bitcast(v, bf16)


def _kernel(x_hbm, wa_hbm, woa_hbm, wb_hbm, wob_hbm, gw_hbm, o_ref,
            x_scr, wa_ref, woa_ref, wb_ref, wob_ref, gw_ref, x_sem, w_sem,
            k_scr, vt_scr, q_scr, ot_scr, wtf_scr, wtp_scr, wobp_scr, qb_scr, kb_scr, vb_scr, ob_scr, g_scr, os_scr, acc_scr):
    step = pl.program_id(0)

    def x_copy(i):
        return pltpu.make_async_copy(x_hbm.at[i], x_scr.at[i], x_sem.at[i])

    def wa_copy(p):
        return pltpu.make_async_copy(wa_hbm.at[:, p * D:(p + 1) * D], wa_ref.at[:, p * D:(p + 1) * D], w_sem.at[p])

    def wa_cols(i):
        c0, c1 = WA_CH[i]
        return pltpu.make_async_copy(wa_hbm.at[:, c0:c1], wa_ref.at[:, c0:c1], w_sem.at[9 + i])

    def wb_copy(p):
        return pltpu.make_async_copy(wb_hbm.at[:, p * D:(p + 1) * D], wb_ref.at[:, p * D:(p + 1) * D], w_sem.at[3 + p])

    woa_copy = pltpu.make_async_copy(woa_hbm, woa_ref, w_sem.at[6])
    wob_copy = pltpu.make_async_copy(wob_hbm, wob_ref, w_sem.at[7])
    gw_copy = pltpu.make_async_copy(gw_hbm, gw_ref, w_sem.at[8])

    def prep_blk(p, j, dep=None):
        jj = j + 5 * (p % 2)
        w = wb_ref[128 * j:128 * j + 128, p * D:(p + 1) * D].astype(f32)
        if dep is not None:
            never = jax.lax.broadcasted_iota(jnp.int32, (8, 128), 0) + step < 0
            top = jnp.concatenate([jnp.where(never, dep, w[0:8, 128 * c:128 * c + 128]) for c in range(5)], axis=1)
            w = jnp.concatenate([top, w[8:]], axis=0)
        wtf_scr[jj] = w.T
        for d in range(DH):
            r = (p * D + H * d) // 2
            wtp_scr[r:r + H // 2, 128 * j:128 * j + 128] = _pack16(wtf_scr[jj, pl.ds(d, H, stride=DH), :])

    def prep_wb(p):
        for j in range(5):
            prep_blk(p, j)

    def prep_wob():
        for j in range(5):
            wtf_scr[j] = wob_ref[:, 128 * j:128 * j + 128].astype(f32)
            for d in range(DH):
                r = H * d // 2
                wobp_scr[r:r + H // 2, 128 * j:128 * j + 128] = _pack16(wtf_scr[j, pl.ds(d, H, stride=DH), :])

    def body(kind):
        first = kind == 0
        last = kind == 2
        if first:
            x_copy(0).start()
            wa_cols(0).start()
            gw_copy.start()
            for i in range(1, 4):
                wa_cols(i).start()
            for p in range(3):
                wb_copy(p).start()
            woa_copy.start()
            wob_copy.start()
            x_copy(1).start()
            kb_scr[0, :, 0:HIST, :] = jnp.zeros((5, HIST, 128), f32)
            vb_scr[0, :, 0:HIST, :] = jnp.zeros((5, HIST, 128), f32)
            x_copy(0).wait()
            gw_copy.wait()
            x_ref = x_scr.at[0]
        else:
            if not last:
                x_copy(step).wait()

                @pl.when(step < LAST)
                def _():
                    x_copy(step + 1).start()

                x_ref = x_scr.at[step]
                k_scr[:, 0:PAD // 2, :] = k_scr[:, TQ // 2:(TQ + PAD) // 2, :]
                vt_scr[:, :, 0:PAD] = vt_scr[:, :, TQ:TQ + PAD]
            o_ref[0:SUB, :] = os_scr[...]

        never = jax.lax.broadcasted_iota(jnp.int32, (BCH, 128), 0) + step < 0
        gw = gw_ref[...].astype(f32)

        def set_gate(sb, xs):
            gate = jax.nn.sigmoid(jnp.sum(xs * gw, axis=1, keepdims=True))
            g_scr[sb * SUB:(sb + 1) * SUB, :] = jnp.broadcast_to(gate, (SUB, 128))

        if not first:
            set_gate(1, x_scr[LAST if last else step - 1, SUB:TQ, :].astype(f32))
        if not last:
            x = x_ref[...]
            xf = x.astype(f32)
            set_gate(0, xf[0:SUB])
            xp = _bf(_pack16(xf))
            xu = pltpu.bitcast(x, u32)
            x_ev = pltpu.unpack_elementwise(xu, index=0, packed_dtype=bf16, unpacked_dtype=f32)
            x_od = pltpu.unpack_elementwise(xu, index=1, packed_dtype=bf16, unpacked_dtype=f32)
            xe = jnp.concatenate([t[8 * i:8 * i + 8] for i in range(TQ // 16) for t in (x_ev, x_od)],
                                 axis=0).astype(bf16)

        def pb(sb, n0, n1):
            rs = slice(sb * SUB, (sb + 1) * SUB)
            res = jax.lax.dot_general(x[rs], _bf(wtp_scr[64 * n0:64 * n1, :]), NT, preferred_element_type=f32)
            for n in range(n0, n1):
                p, c = divmod(n, 5)
                v = res[:, 128 * (n - n0):128 * (n - n0) + 128]
                if p == 0:
                    qb_scr[c, rs, :] = v * QSCALE
                else:
                    dst = kb_scr if p == 1 else vb_scr
                    dst[sb, c, HIST:HIST + SUB, :] = v
                    dst[1 - sb, c, 0:HIST, :] = v[SUB - HIST:SUB]

        def b_chunk(sb, ci, dep):
            r0 = ci * BCH
            R0 = sb * SUB + r0
            qb = [qb_scr[c, R0:R0 + BCH, :] for c in range(5)]
            if dep is not None:
                qb = [jnp.where(never, dep, q) for q in qb]
            logits = []
            for w in range(W_B):
                off = HIST - DIL * w + r0
                acc = qb[0] * kb_scr[sb, 0, off:off + BCH, :]
                for c in range(1, 5):
                    acc = acc + qb[c] * kb_scr[sb, c, off:off + BCH, :]
                acc = acc + pltpu.roll(acc, 64, 1)
                acc = acc + pltpu.roll(acc, 32, 1)
                if first and r0 < DIL * w:
                    pos = r0 + jax.lax.broadcasted_iota(jnp.int32, (BCH, 128), 0)
                    acc = jnp.where(pos >= DIL * w, acc, NEG)
                logits.append(acc)
            m = functools.reduce(jnp.maximum, logits)
            es = [jnp.exp2(l - m) for l in logits]
            den = functools.reduce(lambda a, b: a + b, es)
            fac = (1.0 - g_scr[R0:R0 + BCH, :]) / den
            for c in range(5):
                acc = None
                for w in range(W_B):
                    off = HIST - DIL * w + r0
                    term = es[w] * vb_scr[sb, c, off:off + BCH, :]
                    acc = term if acc is None else acc + term
                acc = acc * fac
                ob_scr[R0:R0 + BCH, 128 * c:128 * c + 128] = acc.astype(bf16)
            return acc

        deps = []

        def attn_b(sb, chain):
            for ci in range(SUB // BCH):
                deps.append(b_chunk(sb, ci, deps[-chain] if chain and len(deps) >= chain else None))

        def emit(sb, v, init, last):
            rs = slice(sb * SUB, (sb + 1) * SUB)
            if not init:
                v = acc_scr[rs, :] + v
            if last:
                if sb == 0:
                    os_scr[...] = v.astype(bf16)
                else:
                    o_ref[rs, :] = v.astype(o_ref.dtype)
            else:
                acc_scr[rs, :] = v

        def op_b(sb, init=False, last=False):
            rs = slice(sb * SUB, (sb + 1) * SUB)
            emit(sb, jnp.dot(ob_scr[rs, :], _bf(wobp_scr[...]), preferred_element_type=f32), init, last)

        def op_b_rows(r0, r1):
            v = jnp.dot(ob_scr[r0:r1, :], _bf(wobp_scr[...]), preferred_element_type=f32)
            o_ref[r0:r1, :] = (acc_scr[r0:r1, :] + v).astype(o_ref.dtype)

        def op_a(sb, c0, c1, init=False, last=False):
            rs = slice(sb * SUB, (sb + 1) * SUB)
            gg = g_scr[rs, :]
            oa = ot_scr[128 * c0:128 * c1, rs].T
            oa = jnp.concatenate([oa[:, 128 * c:128 * c + 128] * gg for c in range(c1 - c0)], axis=1).astype(bf16)
            emit(sb, jnp.dot(oa, woa_ref[128 * c0:128 * c1, :], preferred_element_type=f32), init, last)

        def dot_a(p):
            return jnp.dot(xp if p == 2 else xe, wa_ref[:, p * D:(p + 1) * D], preferred_element_type=f32)

        def dot_c(c0, c1):
            return jnp.dot(xp if c0 >= 2 * D else xe, wa_ref[:, c0:c1], preferred_element_type=f32)

        def post_v(va):
            vat = va.T
            rid = jax.lax.broadcasted_iota(jnp.int32, (32, TQ), 0)
            for h in range(H):
                base, o, r = _vwin(h)
                win = jnp.where(rid == r, 1.0, vat[base:base + 32, :])
                vt_scr[h, :, PAD:PAD + TQ] = win.astype(bf16)

        def post_k(ka):
            for g in range(NG):
                k_scr[g, PAD // 2:(PAD + TQ) // 2, :] = _pack16(ka[:, G_OFF[g]:G_OFF[g] + 128])

        def post_q(qa):
            qa = qa * QSCALE
            for g in range(NG):
                q_scr[g] = _pack16(qa[:, G_OFF[g]:G_OFF[g] + 128])

        lane = jax.lax.broadcasted_iota(jnp.int32, (QB, 128), 1)
        krow = jax.lax.broadcasted_iota(jnp.int32, (QB, 128), 0)
        old_valid = krow > (lane & (QB - 1))
        lane16 = jax.lax.broadcasted_iota(jnp.int32, (QB // 2, 128), 1)

        def masks(rows):
            slot = jax.lax.broadcasted_iota(jnp.int32, (rows, 128), 1) // QB
            return slot, (slot == 0) | (slot == 2), slot < 2, (slot == 1) | (slot == 2)

        mk16 = masks(QB // 2)
        mk1 = masks(1)

        def butterfly(X, mk):
            slot, m_even, m_01, m_12 = mk

            def sel(m, a, b):
                if a is None and b is None:
                    return None
                z = jnp.zeros_like(a if b is None else b)
                return jnp.where(m, z if a is None else a, z if b is None else b)

            live = [t for t in range(GH) if X[t] is not None]
            if len(live) == 1:
                t = live[0]
                return [sel(slot == (j + t) % GH, X[t], None) for j in range(GH)]
            a0 = sel(m_even, X[0], X[1])
            a1 = sel(m_even, X[1], X[0])
            b0 = sel(m_even, X[2], X[3])
            b1 = sel(m_even, X[3], X[2])
            return [sel(m_01, a0, b0), sel(m_12, a1, b1), sel(m_01, b0, a0), sel(m_12, b1, a1)]

        st8 = {}

        def segs_of(idx):
            sb = idx // NG
            return tuple(range(2 - sb, 3)) if first else (0, 1, 2)

        def qweights(idx, t):
            sb, g = divmod(idx, NG)
            r0 = (sb * SUB + QB * t) // 2
            q = q_scr[g, r0:r0 + QB // 2, :]
            parts = []
            for s in range(GH):
                j = (s - t) % GH
                lo = DH * (GH * g + j) - G_OFF[g]
                parts.append(jnp.where((lane16 >= lo) & (lane16 < lo + DH), q, jnp.zeros_like(q)))
            return _bf(jnp.concatenate(parts, axis=0))

        def seg_range(t, seg):
            return max(4 * seg - t, 0), min(4 * seg + 4 - t, NU)

        def soft(idx, t, seg, chunks):
            S_ = st8.setdefault(idx, {'P': [dict() for _ in range(GH)], 'm': {}, 'o': {}})
            u0, u1 = seg_range(t, seg)
            ss = {}
            for u in range(u0, u1):
                s = chunks[u]
                if u == 0:
                    s = jnp.where(old_valid, s, NEG)
                if u == NU - 1:
                    s = jnp.where(old_valid, NEG, s)
                ss[u] = s
            mx = functools.reduce(jnp.maximum,
                                  [ss[u][8 * i:8 * i + 8] for u in range(u0, u1) for i in range(QB // 8)])
            m = jnp.max(mx, axis=0, keepdims=True)
            S_['m'][(t, seg)] = m
            for u in range(u0, u1):
                S_['P'][t][u] = _pack16(jnp.exp2(ss[u] - m))

        def qk(idx):
            sb, g = divmod(idx, NG)
            segs = segs_of(idx)
            chunks = []
            for t in range(GH):
                u0 = seg_range(t, segs[0])[0]
                r0 = (sb * SUB + QB * t) // 2
                kk = _bf(k_scr[g, r0 + u0 * QB // 2:r0 + NU * QB // 2, :])
                st = jax.lax.dot_general(kk, qweights(idx, t), NT, preferred_element_type=f32)
                chunks.append({u: st[QB * (u - u0):QB * (u - u0) + QB] for u in range(u0, NU)})
            for seg in segs:
                for t in ((3, 2, 1, 0) if seg < 2 else (0, 1, 2, 3)):
                    soft(idx, t, seg, chunks[t])

        def pv(idx):
            sb, g = divmod(idx, NG)
            segs = segs_of(idx)
            S_ = st8.pop(idx)
            for seg in segs:
                outs = [[] for _ in range(GH)]
                for c in range(4 * seg, 4 * seg + 4):
                    X = [S_['P'][t].get(c - t) for t in range(GH)]
                    for j, v in enumerate(butterfly(X, mk16)):
                        outs[j].append(v)
                for j in range(GH):
                    h = GH * g + j
                    pt = _bf(jnp.concatenate(outs[j], axis=0))
                    vt = vt_scr[h, :, (sb + seg) * SUB:(sb + seg + 1) * SUB]
                    S_['o'][(j, seg)] = jnp.dot(vt, pt, preferred_element_type=f32)
            al = {}
            if len(segs) > 1:
                mf = [functools.reduce(jnp.maximum, [S_['m'][(t, seg)] for seg in segs]) for t in range(GH)]
                for seg in segs:
                    al[seg] = butterfly([jnp.exp2(S_['m'][(t, seg)] - mf[t]) for t in range(GH)], mk1)
            for j in range(GH):
                h = GH * g + j
                if len(segs) > 1:
                    ot = functools.reduce(lambda a, b: a + b, [S_['o'][(j, seg)] * al[seg][j] for seg in segs])
                else:
                    ot = S_['o'][(j, segs[0])]
                base, o, r = _vwin(h)
                inv = 1.0 / ot[r:r + 1, :]
                on = ot * inv
                if j:
                    on = pltpu.roll(on, 128 - QB * j, 1)
                ot_scr[DH * h:DH * h + DH, sb * SUB:(sb + 1) * SUB] = on[o:o + DH, :]
            return on[0:8]

        nidx = NSB * NG

        def attn(i0, i1):
            for idx in range(i0, i1):
                if idx < nidx:
                    qk(idx)
                if idx > 0:
                    pv(idx - 1)

        if first:
            wa_copy_dummy = None
            wa_cols(0).wait()
            v1 = dot_c(1408, 1920)
            wa_cols(1).wait()
            v0 = dot_c(1280, 1408)
            k1 = dot_c(896, 1280)
            post_v(jnp.concatenate([v0, v1], axis=1))
            wa_cols(2).wait()
            k0 = dot_c(640, 896)
            q1 = dot_c(384, 640)
            post_k(jnp.concatenate([k0, k1], axis=1))
            wa_cols(3).wait()
            q0 = dot_c(0, 384)
            post_q(jnp.concatenate([q0, q1], axis=1))
            seq = [8, 0, 9, 1, 10, 2, 11, 3, 12, 4, 13, 5, 14, 6, 15, 7]
            qk(seq[0])
            qk(seq[1])
            wb_copy(0).wait()
            tie = {2: 0, 4: 1, 6: 2, 8: 3, 10: 4}
            if 0 not in tie.values():
                prep_blk(0, 0)
            for i, idx in enumerate(seq):
                if i > 1:
                    qk(idx)
                    dep = pv(seq[i - 2])
                    if i in tie:
                        prep_blk(0, tie[i], dep)
            pb(0, 0, 2)
            pv(seq[-2])
            pb(0, 2, 3)
            pv(seq[-1])
            pb(0, 3, 4)
            wb_copy(1).wait()
            wb_copy(2).wait()
            prep_wb(1)
            prep_wb(2)
            pb(0, 4, 5)
            pb(1, 0, 5)
            pb(0, 5, 10)
            pb(0, 10, 15)
            wob_copy.wait()
            woa_copy.wait()
            attn_b(0, 8)
            prep_wob()
            pb(1, 5, 15)
            op_a(0, 0, 5, init=True)
            op_b(0, last=True)
        elif last:
            attn_b(1, 0)
            oa = ot_scr[:, SUB:TQ].T.astype(bf16)
            va = jnp.dot(oa, woa_ref[...], preferred_element_type=f32)
            for r0, r1 in ((0, 32), (32, 64), (64, 96), (96, 128)):
                vb = jnp.dot(ob_scr[SUB + r0:SUB + r1, :], _bf(wobp_scr[...]), preferred_element_type=f32)
                gg = g_scr[SUB + r0:SUB + r1, :]
                v = jnp.concatenate([va[r0:r1, 128 * c:128 * c + 128] * gg for c in range(5)], axis=1) + vb
                o_ref[SUB + r0:SUB + r1, :] = v.astype(o_ref.dtype)
        else:
            attn_b(1, BCHAIN)
            pb(0, 0, 15)
            attn_b(0, BCHAIN)
            post_v(dot_a(2))
            op_a(1, 0, 5, init=True)
            post_k(dot_a(1))
            op_b(1, last=True)
            post_q(dot_a(0))
            op_b(0, init=True)
            fill = {1: (0, 2), 3: (2, 4), 5: (4, 6), 7: (6, 8), 9: (8, 9), 13: (9, 10), 15: (10, 13), 16: (13, 15)}
            for idx in range(nidx + 1):
                attn(idx, idx + 1)
                if idx in fill:
                    pb(1, *fill[idx])
                if idx == 11:
                    op_a(0, 0, 5, last=True)

    @pl.when(step == 0)
    def _():
        body(0)

    @pl.when((step > 0) & (step < NSTEP))
    def _():
        body(1)

    @pl.when(step == NSTEP)
    def _():
        body(2)


@jax.jit
def pallas_gated_mix__sliding_block__sliding_local_dilated__prompt_kernel(A_x, A_wqkv, A_wo, B_x, B_wqkv, B_wo, gate_w):
    x = A_x.reshape(NSTEP, TQ, D)
    gw = gate_w.reshape(1, D)
    hbm = pl.BlockSpec(memory_space=pl.ANY)
    out = pl.pallas_call(
        _kernel,
        grid=(NSTEP + 1,),
        in_specs=[hbm] * 6,
        out_specs=pl.BlockSpec((TQ, D), lambda i: (jnp.maximum(i - 1, 0), 0)),
        out_shape=jax.ShapeDtypeStruct((S, D), bf16),
        scratch_shapes=[
            pltpu.VMEM((NSTEP, TQ, D), bf16),
            pltpu.VMEM((D, 3 * D), bf16),
            pltpu.VMEM((D, D), bf16),
            pltpu.VMEM((D, 3 * D), bf16),
            pltpu.VMEM((D, D), bf16),
            pltpu.VMEM((1, D), bf16),
            pltpu.SemaphoreType.DMA((NSTEP,)),
            pltpu.SemaphoreType.DMA((13,)),
            pltpu.VMEM((NG, (PAD + TQ) // 2, 128), u32),
            pltpu.VMEM((H, 32, PAD + TQ), bf16),
            pltpu.VMEM((NG, TQ // 2, 128), u32),
            pltpu.VMEM((D, TQ), f32),
            pltpu.VMEM((10, D, 128), f32),
            pltpu.VMEM((3 * D // 2, D), u32),
            pltpu.VMEM((D // 2, D), u32),
            pltpu.VMEM((5, TQ, 128), f32),
            pltpu.VMEM((NSB, 5, HIST + SUB, 128), f32),
            pltpu.VMEM((NSB, 5, HIST + SUB, 128), f32),
            pltpu.VMEM((TQ, D), bf16),
            pltpu.VMEM((TQ, 128), f32),
            pltpu.VMEM((SUB, D), bf16),
            pltpu.VMEM((TQ, D), f32),
        ],
        compiler_params=pltpu.CompilerParams(
            dimension_semantics=("arbitrary",),
            vmem_limit_bytes=100 * 1024 * 1024,
        ),
    )(x, A_wqkv, A_wo, B_wqkv, B_wo, gw)
    return out.reshape(1, S, D)
```

```python
import functools
import jax
import jax.numpy as jnp
import jax.experimental.pallas as pl
import jax.experimental.pallas.tpu as pltpu

S = 2048
D = 640
H = 32
DH = 20
W_B = 8
DIL = 2
TQ = 256
NSTEP = S // TQ
SUB = 128
NSB = TQ // SUB
LAST = NSTEP - 1
PAD = 256
LOG2E = 1.4426950408889634
QSCALE = (DH ** -0.5) * LOG2E
NEG = -1e9
HIST = 16
NG = 8
GH = 4
QB = 32
NU = PAD // QB + 1
G_OFF = (0, 64, 128, 192, 320, 384, 448, 512)
BCH = 8
BCHAIN = 2
BCHAIN0 = 4
WA_CH = ((1408, 1920), (896, 1408), (384, 896), (0, 384))

f32, bf16, u32 = jnp.float32, jnp.bfloat16, jnp.uint32
NT = (((1,), (1,)), ((), ()))


def _vwin(h):
    base = 16 * ((DH * h) // 16)
    o = DH * h - base
    r = o + DH if o + DH < 32 else 0
    return base, o, r


def _pack16(v):
    n = v.shape[0] // 16
    lo = jnp.concatenate([v[16 * i:16 * i + 8] for i in range(n)], axis=0)
    hi = jnp.concatenate([v[16 * i + 8:16 * i + 16] for i in range(n)], axis=0)
    return pltpu.pack_elementwise([lo, hi], packed_dtype=bf16).astype(u32)


def _bf(v):
    return pltpu.bitcast(v, bf16)


def _kernel(x_hbm, wa_hbm, woa_hbm, wb_hbm, wob_hbm, gw_hbm, o_ref,
            x_scr, wa_ref, woa_ref, wb_ref, wob_ref, gw_ref, x_sem, w_sem,
            k_scr, vt_scr, q_scr, ot_scr, wtf_scr, wtp_scr, wobp_scr, qb_scr, kb_scr, vb_scr, ob_scr, g_scr, os_scr, o_sem, acc_scr):
    step = pl.program_id(0)

    def x_copy(i):
        return pltpu.make_async_copy(x_hbm.at[i], x_scr.at[i], x_sem.at[i % 2])

    def wa_cols(i):
        c0, c1 = WA_CH[i]
        return pltpu.make_async_copy(wa_hbm.at[:, c0:c1], wa_ref.at[:, c0:c1], w_sem.at[(0, 1, 2, 9)[i]])

    def wb_copy(p):
        return pltpu.make_async_copy(wb_hbm.at[:, p * D:(p + 1) * D], wb_ref.at[:, p * D:(p + 1) * D], w_sem.at[3 + p])

    def o_copy(q, n):
        return pltpu.make_async_copy(os_scr.at[pl.ds(q, n)], o_ref.at[pl.ds(q, n)], o_sem.at[n % 2])

    woa_copy = pltpu.make_async_copy(woa_hbm, woa_ref, w_sem.at[6])
    wob_copy = pltpu.make_async_copy(wob_hbm, wob_ref, w_sem.at[7])
    gw_copy = pltpu.make_async_copy(gw_hbm, gw_ref, w_sem.at[8])

    def prep_blk(p, j, dep=None):
        jj = j + 5 * (p % 2)
        w = wb_ref[128 * j:128 * j + 128, p * D:(p + 1) * D].astype(f32)
        if dep is not None:
            never = jax.lax.broadcasted_iota(jnp.int32, (8, 128), 0) + step < 0
            top = jnp.concatenate([jnp.where(never, dep, w[0:8, 128 * c:128 * c + 128]) for c in range(5)], axis=1)
            w = jnp.concatenate([top, w[8:]], axis=0)
        wtf_scr[jj] = w.T
        for d in range(DH):
            r = (p * D + H * d) // 2
            wtp_scr[r:r + H // 2, 128 * j:128 * j + 128] = _pack16(wtf_scr[jj, pl.ds(d, H, stride=DH), :])

    def prep_wb(p):
        for j in range(5):
            prep_blk(p, j)

    def prep_wob():
        for j in range(5):
            wtf_scr[j] = wob_ref[:, 128 * j:128 * j + 128].astype(f32)
            for d in range(DH):
                r = H * d // 2
                wobp_scr[r:r + H // 2, 128 * j:128 * j + 128] = _pack16(wtf_scr[j, pl.ds(d, H, stride=DH), :])

    def body(kind):
        first = kind == 0
        last = kind == 2
        if first:
            x_copy(0).start()
            wa_cols(0).start()
            gw_copy.start()
            for i in range(1, 4):
                wa_cols(i).start()
            for p in range(3):
                wb_copy(p).start()
            woa_copy.start()
            wob_copy.start()
            x_copy(1).start()
            kb_scr[0, :, 0:HIST, :] = jnp.zeros((5, HIST, 128), f32)
            vb_scr[0, :, 0:HIST, :] = jnp.zeros((5, HIST, 128), f32)
            x_copy(0).wait()
            gw_copy.wait()
            x_ref = x_scr.at[0]
        else:
            if not last:
                x_copy(step).wait()

                @pl.when(step < LAST)
                def _():
                    x_copy(step + 1).start()

                x_ref = x_scr.at[step]
                k_scr[:, 0:PAD // 2, :] = k_scr[:, TQ // 2:(TQ + PAD) // 2, :]
                vt_scr[:, :, 0:PAD] = vt_scr[:, :, TQ:TQ + PAD]

        never = jax.lax.broadcasted_iota(jnp.int32, (BCH, 128), 0) + step < 0
        gw = gw_ref[...].astype(f32)

        def set_gate(sb, xs):
            gate = jax.nn.sigmoid(jnp.sum(xs * gw, axis=1, keepdims=True))
            g_scr[sb * SUB:(sb + 1) * SUB, :] = jnp.broadcast_to(gate, (SUB, 128))

        if not first:
            set_gate(1, x_scr[LAST if last else step - 1, SUB:TQ, :].astype(f32))
        if not last:
            x = x_ref[...]
            xf = x.astype(f32)
            set_gate(0, xf[0:SUB])
            xp = _bf(_pack16(xf))
            xu = pltpu.bitcast(x, u32)
            x_ev = pltpu.unpack_elementwise(xu, index=0, packed_dtype=bf16, unpacked_dtype=f32)
            x_od = pltpu.unpack_elementwise(xu, index=1, packed_dtype=bf16, unpacked_dtype=f32)
            xe = jnp.concatenate([t[8 * i:8 * i + 8] for i in range(TQ // 16) for t in (x_ev, x_od)],
                                 axis=0).astype(bf16)

        def pb(sb, n0, n1):
            rs = slice(sb * SUB, (sb + 1) * SUB)
            res = jax.lax.dot_general(x[rs], _bf(wtp_scr[64 * n0:64 * n1, :]), NT, preferred_element_type=f32)
            for n in range(n0, n1):
                p, c = divmod(n, 5)
                v = res[:, 128 * (n - n0):128 * (n - n0) + 128]
                if p == 0:
                    qb_scr[c, rs, :] = v * QSCALE
                else:
                    dst = kb_scr if p == 1 else vb_scr
                    dst[sb, c, HIST:HIST + SUB, :] = v
                    dst[1 - sb, c, 0:HIST, :] = v[SUB - HIST:SUB]

        def b_chunk(sb, ci, dep):
            r0 = ci * BCH
            R0 = sb * SUB + r0
            qb = [qb_scr[c, R0:R0 + BCH, :] for c in range(5)]
            if dep is not None:
                qb = [jnp.where(never, dep, q) for q in qb]
            logits = []
            for w in range(W_B):
                off = HIST - DIL * w + r0
                acc = qb[0] * kb_scr[sb, 0, off:off + BCH, :]
                for c in range(1, 5):
                    acc = acc + qb[c] * kb_scr[sb, c, off:off + BCH, :]
                acc = acc + pltpu.roll(acc, 64, 1)
                acc = acc + pltpu.roll(acc, 32, 1)
                if first and r0 < DIL * w:
                    pos = r0 + jax.lax.broadcasted_iota(jnp.int32, (BCH, 128), 0)
                    acc = jnp.where(pos >= DIL * w, acc, NEG)
                logits.append(acc)
            m = functools.reduce(jnp.maximum, logits)
            es = [jnp.exp2(l - m) for l in logits]
            den = functools.reduce(lambda a, b: a + b, es)
            fac = (1.0 - g_scr[R0:R0 + BCH, :]) / den
            for c in range(5):
                acc = None
                for w in range(W_B):
                    off = HIST - DIL * w + r0
                    term = es[w] * vb_scr[sb, c, off:off + BCH, :]
                    acc = term if acc is None else acc + term
                acc = acc * fac
                ob_scr[R0:R0 + BCH, 128 * c:128 * c + 128] = acc.astype(bf16)
            return acc

        deps = []

        def attn_b(sb, chain):
            for ci in range(SUB // BCH):
                deps.append(b_chunk(sb, ci, deps[-chain] if chain and len(deps) >= chain else None))

        def emit(sb, v, init, last):
            rs = slice(sb * SUB, (sb + 1) * SUB)
            if not init:
                v = acc_scr[rs, :] + v
            if last:
                q0 = 0 if first else 8 * step - 4 * sb
                os_scr[pl.ds(q0, 4)] = v.astype(bf16).reshape(4, 32, D)
                o_copy(q0, 4).start()
            else:
                acc_scr[rs, :] = v

        def op_b(sb, init=False, last=False):
            rs = slice(sb * SUB, (sb + 1) * SUB)
            emit(sb, jnp.dot(ob_scr[rs, :], _bf(wobp_scr[...]), preferred_element_type=f32), init, last)

        def op_b_rows(r0, r1):
            v = jnp.dot(ob_scr[r0:r1, :], _bf(wobp_scr[...]), preferred_element_type=f32)
            o_ref[r0:r1, :] = (acc_scr[r0:r1, :] + v).astype(o_ref.dtype)

        def op_a(sb, c0, c1, init=False, last=False):
            rs = slice(sb * SUB, (sb + 1) * SUB)
            gg = g_scr[rs, :]
            oa = ot_scr[128 * c0:128 * c1, rs].T
            oa = jnp.concatenate([oa[:, 128 * c:128 * c + 128] * gg for c in range(c1 - c0)], axis=1).astype(bf16)
            emit(sb, jnp.dot(oa, woa_ref[128 * c0:128 * c1, :], preferred_element_type=f32), init, last)

        def dot_a(p):
            return jnp.dot(xp if p == 2 else xe, wa_ref[:, p * D:(p + 1) * D], preferred_element_type=f32)

        def dot_c(c0, c1):
            return jnp.dot(xp if c0 >= 2 * D else xe, wa_ref[:, c0:c1], preferred_element_type=f32)

        def post_v(va):
            vat = va.T
            rid = jax.lax.broadcasted_iota(jnp.int32, (32, TQ), 0)
            for h in range(H):
                base, o, r = _vwin(h)
                win = jnp.where(rid == r, 1.0, vat[base:base + 32, :])
                vt_scr[h, :, PAD:PAD + TQ] = win.astype(bf16)

        def post_k(ka):
            for g in range(NG):
                k_scr[g, PAD // 2:(PAD + TQ) // 2, :] = _pack16(ka[:, G_OFF[g]:G_OFF[g] + 128])

        def post_q(qa):
            qa = qa * QSCALE
            for g in range(NG):
                q_scr[g] = _pack16(qa[:, G_OFF[g]:G_OFF[g] + 128])

        lane = jax.lax.broadcasted_iota(jnp.int32, (QB, 128), 1)
        krow = jax.lax.broadcasted_iota(jnp.int32, (QB, 128), 0)
        old_valid = krow > (lane & (QB - 1))
        lane16 = jax.lax.broadcasted_iota(jnp.int32, (QB // 2, 128), 1)

        def masks(rows):
            slot = jax.lax.broadcasted_iota(jnp.int32, (rows, 128), 1) // QB
            return slot, (slot == 0) | (slot == 2), slot < 2, (slot == 1) | (slot == 2)

        mk16 = masks(QB // 2)
        mk1 = masks(1)

        def butterfly(X, mk):
            slot, m_even, m_01, m_12 = mk

            def sel(m, a, b):
                if a is None and b is None:
                    return None
                z = jnp.zeros_like(a if b is None else b)
                return jnp.where(m, z if a is None else a, z if b is None else b)

            live = [t for t in range(GH) if X[t] is not None]
            if len(live) == 1:
                t = live[0]
                return [sel(slot == (j + t) % GH, X[t], None) for j in range(GH)]
            a0 = sel(m_even, X[0], X[1])
            a1 = sel(m_even, X[1], X[0])
            b0 = sel(m_even, X[2], X[3])
            b1 = sel(m_even, X[3], X[2])
            return [sel(m_01, a0, b0), sel(m_12, a1, b1), sel(m_01, b0, a0), sel(m_12, b1, a1)]

        st8 = {}

        def segs_of(idx):
            sb = idx // NG
            return tuple(range(2 - sb, 3)) if first else (0, 1, 2)

        def qweights(idx, t):
            sb, g = divmod(idx, NG)
            r0 = (sb * SUB + QB * t) // 2
            q = q_scr[g, r0:r0 + QB // 2, :]
            parts = []
            for s in range(GH):
                j = (s - t) % GH
                lo = DH * (GH * g + j) - G_OFF[g]
                parts.append(jnp.where((lane16 >= lo) & (lane16 < lo + DH), q, jnp.zeros_like(q)))
            return _bf(jnp.concatenate(parts, axis=0))

        def seg_range(t, seg):
            return max(4 * seg - t, 0), min(4 * seg + 4 - t, NU)

        def soft(idx, t, seg, chunks):
            S_ = st8.setdefault(idx, {'P': [dict() for _ in range(GH)], 'm': {}, 'o': {}})
            u0, u1 = seg_range(t, seg)
            ss = {}
            for u in range(u0, u1):
                s = chunks[u]
                if u == 0:
                    s = jnp.where(old_valid, s, NEG)
                if u == NU - 1:
                    s = jnp.where(old_valid, NEG, s)
                ss[u] = s
            mx = functools.reduce(jnp.maximum,
                                  [ss[u][8 * i:8 * i + 8] for u in range(u0, u1) for i in range(QB // 8)])
            m = jnp.max(mx, axis=0, keepdims=True)
            S_['m'][(t, seg)] = m
            for u in range(u0, u1):
                S_['P'][t][u] = _pack16(jnp.exp2(ss[u] - m))

        def qk(idx):
            sb, g = divmod(idx, NG)
            segs = segs_of(idx)
            chunks = []
            for t in range(GH):
                u0 = seg_range(t, segs[0])[0]
                r0 = (sb * SUB + QB * t) // 2
                kk = _bf(k_scr[g, r0 + u0 * QB // 2:r0 + NU * QB // 2, :])
                st = jax.lax.dot_general(kk, qweights(idx, t), NT, preferred_element_type=f32)
                chunks.append({u: st[QB * (u - u0):QB * (u - u0) + QB] for u in range(u0, NU)})
            for seg in segs:
                for t in ((3, 2, 1, 0) if seg < 2 else (0, 1, 2, 3)):
                    soft(idx, t, seg, chunks[t])

        def pv(idx):
            sb, g = divmod(idx, NG)
            segs = segs_of(idx)
            S_ = st8.pop(idx)
            for seg in segs:
                outs = [[] for _ in range(GH)]
                for c in range(4 * seg, 4 * seg + 4):
                    X = [S_['P'][t].get(c - t) for t in range(GH)]
                    for j, v in enumerate(butterfly(X, mk16)):
                        outs[j].append(v)
                for j in range(GH):
                    h = GH * g + j
                    pt = _bf(jnp.concatenate(outs[j], axis=0))
                    vt = vt_scr[h, :, (sb + seg) * SUB:(sb + seg + 1) * SUB]
                    S_['o'][(j, seg)] = jnp.dot(vt, pt, preferred_element_type=f32)
            al = {}
            if len(segs) > 1:
                mf = [functools.reduce(jnp.maximum, [S_['m'][(t, seg)] for seg in segs]) for t in range(GH)]
                for seg in segs:
                    al[seg] = butterfly([jnp.exp2(S_['m'][(t, seg)] - mf[t]) for t in range(GH)], mk1)
            for j in range(GH):
                h = GH * g + j
                if len(segs) > 1:
                    ot = functools.reduce(lambda a, b: a + b, [S_['o'][(j, seg)] * al[seg][j] for seg in segs])
                else:
                    ot = S_['o'][(j, segs[0])]
                base, o, r = _vwin(h)
                inv = 1.0 / ot[r:r + 1, :]
                on = ot * inv
                if j:
                    on = pltpu.roll(on, 128 - QB * j, 1)
                ot_scr[DH * h:DH * h + DH, sb * SUB:(sb + 1) * SUB] = on[o:o + DH, :]
            return on[0:8]

        nidx = NSB * NG

        def attn(i0, i1):
            for idx in range(i0, i1):
                if idx < nidx:
                    qk(idx)
                if idx > 0:
                    pv(idx - 1)

        if first:
            wa_copy_dummy = None
            wa_cols(0).wait()
            v1 = dot_c(1408, 1920)
            wa_cols(1).wait()
            v0 = dot_c(1280, 1408)
            k1 = dot_c(896, 1280)
            post_v(jnp.concatenate([v0, v1], axis=1))
            wa_cols(2).wait()
            k0 = dot_c(640, 896)
            q1 = dot_c(384, 640)
            post_k(jnp.concatenate([k0, k1], axis=1))
            wa_cols(3).wait()
            q0 = dot_c(0, 384)
            post_q(jnp.concatenate([q0, q1], axis=1))
            seq = [8, 0, 9, 1, 10, 2, 11, 3, 12, 4, 13, 5, 14, 6, 15, 7]
            qk(seq[0])
            qk(seq[1])
            wb_copy(0).wait()
            tie = {2: 0, 4: 1, 6: 2, 8: 3, 10: 4}
            if 0 not in tie.values():
                prep_blk(0, 0)
            for i, idx in enumerate(seq):
                if i > 1:
                    qk(idx)
                    dep = pv(seq[i - 2])
                    if i in tie:
                        prep_blk(0, tie[i], dep)
            pb(0, 0, 2)
            pv(seq[-2])
            pb(0, 2, 3)
            pv(seq[-1])
            pb(0, 3, 4)
            wb_copy(1).wait()
            wb_copy(2).wait()
            prep_wb(1)
            prep_wb(2)
            pb(0, 4, 5)
            pb(1, 0, 5)
            pb(0, 5, 10)
            pb(0, 10, 15)
            wob_copy.wait()
            woa_copy.wait()
            attn_b(0, 8)
            prep_wob()
            pb(1, 5, 15)
            op_a(0, 0, 5, init=True)
            op_b(0, last=True)
        elif last:
            attn_b(1, 0)
            oa = ot_scr[:, SUB:TQ].T.astype(bf16)
            va = jnp.dot(oa, woa_ref[...], preferred_element_type=f32)
            for r0, r1 in ((0, 32), (32, 64), (64, 96), (96, 128)):
                vb = jnp.dot(ob_scr[SUB + r0:SUB + r1, :], _bf(wobp_scr[...]), preferred_element_type=f32)
                gg = g_scr[SUB + r0:SUB + r1, :]
                v = jnp.concatenate([va[r0:r1, 128 * c:128 * c + 128] * gg for c in range(5)], axis=1) + vb
                q0 = S // 32 - 4 + r0 // 32
                os_scr[q0] = v.astype(bf16)
                o_copy(q0, 1).start()
            for q in range(0, S // 32 - 4, 4):
                o_copy(q, 4).wait()
            for q in range(S // 32 - 4, S // 32):
                o_copy(q, 1).wait()
        else:
            attn_b(1, BCHAIN)
            pb(0, 0, 15)
            attn_b(0, BCHAIN)
            post_v(dot_a(2))
            op_a(1, 0, 5, init=True)
            post_k(dot_a(1))
            op_b(1, last=True)
            post_q(dot_a(0))
            op_b(0, init=True)
            fill = {1: (0, 2), 3: (2, 4), 5: (4, 6), 7: (6, 8), 9: (8, 9), 13: (9, 10), 15: (10, 13), 16: (13, 15)}
            for idx in range(nidx + 1):
                attn(idx, idx + 1)
                if idx in fill:
                    pb(1, *fill[idx])
                if idx == 11:
                    op_a(0, 0, 5, last=True)

    @pl.when(step == 0)
    def _():
        body(0)

    @pl.when(step > 0)
    def _():
        body(1)

    @pl.when(step == LAST)
    def _():
        body(2)


@jax.jit
def pallas_gated_mix__sliding_block__sliding_local_dilated__prompt_kernel(A_x, A_wqkv, A_wo, B_x, B_wqkv, B_wo, gate_w):
    x = A_x.reshape(NSTEP, TQ, D)
    gw = gate_w.reshape(1, D)
    hbm = pl.BlockSpec(memory_space=pl.ANY)
    out = pl.pallas_call(
        _kernel,
        grid=(NSTEP,),
        in_specs=[hbm] * 6,
        out_specs=hbm,
        out_shape=jax.ShapeDtypeStruct((S // 32, 32, D), bf16),
        scratch_shapes=[
            pltpu.VMEM((NSTEP, TQ, D), bf16),
            pltpu.VMEM((D, 3 * D), bf16),
            pltpu.VMEM((D, D), bf16),
            pltpu.VMEM((D, 3 * D), bf16),
            pltpu.VMEM((D, D), bf16),
            pltpu.VMEM((1, D), bf16),
            pltpu.SemaphoreType.DMA((2,)),
            pltpu.SemaphoreType.DMA((10,)),
            pltpu.VMEM((NG, (PAD + TQ) // 2, 128), u32),
            pltpu.VMEM((H, 32, PAD + TQ), bf16),
            pltpu.VMEM((NG, TQ // 2, 128), u32),
            pltpu.VMEM((D, TQ), f32),
            pltpu.VMEM((10, D, 128), f32),
            pltpu.VMEM((3 * D // 2, D), u32),
            pltpu.VMEM((D // 2, D), u32),
            pltpu.VMEM((5, TQ, 128), f32),
            pltpu.VMEM((NSB, 5, HIST + SUB, 128), f32),
            pltpu.VMEM((NSB, 5, HIST + SUB, 128), f32),
            pltpu.VMEM((TQ, D), bf16),
            pltpu.VMEM((TQ, 128), f32),
            pltpu.VMEM((S // 32, 32, D), bf16),
            pltpu.SemaphoreType.DMA((2,)),
            pltpu.VMEM((TQ, D), f32),
        ],
        compiler_params=pltpu.CompilerParams(
            dimension_semantics=("arbitrary",),
            vmem_limit_bytes=100 * 1024 * 1024,
        ),
    )(x, A_wqkv, A_wo, B_wqkv, B_wo, gw)
    return out.reshape(1, S, D)
```

```python
import functools
import jax
import jax.numpy as jnp
import jax.experimental.pallas as pl
import jax.experimental.pallas.tpu as pltpu

S = 2048
D = 640
H = 32
DH = 20
W_B = 8
DIL = 2
TQ = 256
NSTEP = S // TQ
SUB = 128
NSB = TQ // SUB
LAST = NSTEP - 1
PAD = 256
LOG2E = 1.4426950408889634
QSCALE = (DH ** -0.5) * LOG2E
NEG = -1e9
HIST = 16
NG = 8
GH = 4
QB = 32
NU = PAD // QB + 1
G_OFF = (0, 64, 128, 192, 320, 384, 448, 512)
VW = 24
QR = GH * DH // 2
BCH = 8
WA_CH = ((0, 128, 0, 640), (0, 128, 640, 1920), (128, 256, 0, 1920), (256, 384, 0, 1920), (384, 640, 1280, 1920),
         (384, 640, 0, 1280))
X0_CH = ((0, 128), (128, 256), (256, 640))

f32, bf16, u32 = jnp.float32, jnp.bfloat16, jnp.uint32
NT = (((1,), (1,)), ((), ()))
NN = (((1,), (0,)), ((), ()))


def _vwin(h):
    base = 8 * ((DH * h) // 8)
    o = DH * h - base
    r = o + DH if o + DH < VW else 0
    return base, o, r


def _pack16(v):
    n = v.shape[0] // 16
    lo = jnp.concatenate([v[16 * i:16 * i + 8] for i in range(n)], axis=0)
    hi = jnp.concatenate([v[16 * i + 8:16 * i + 16] for i in range(n)], axis=0)
    return pltpu.pack_elementwise([lo, hi], packed_dtype=bf16).astype(u32)


def _bf(v):
    return pltpu.bitcast(v, bf16)


def _kernel(x_hbm, wa_hbm, woa_hbm, wb_hbm, wob_hbm, gw_hbm, o_ref,
            x_scr, wa_ref, woa_ref, wb_ref, wob_ref, gw_ref,
            k_scr, vt_scr, q_scr, ot_scr, wtf_scr, wtp_scr, wobp_scr, qb_scr, kb_scr, vb_scr, ob_scr, g_scr,
            os_scr, o_sem, acc_scr, pa_scr, sem, gwf_scr):
    pid = pl.program_id(0)

    x_copy = pltpu.make_async_copy(x_hbm.at[1:LAST], x_scr.at[1:LAST], sem.at[18])

    def wa_cols(i):
        r0, r1, c0, c1 = WA_CH[i]
        return pltpu.make_async_copy(wa_hbm.at[r0:r1, c0:c1], wa_ref.at[r0:r1, c0:c1], sem.at[i])

    def x0_cols(i, far):
        c0, c1 = X0_CH[i]
        b = LAST if far else 0
        return pltpu.make_async_copy(x_hbm.at[b, :, c0:c1], x_scr.at[b, :, c0:c1], sem.at[len(WA_CH) + 2 * i + far])

    def wb_copy(p):
        cs = slice(D, 3 * D) if p else slice(0, D)
        return pltpu.make_async_copy(wb_hbm.at[:, cs], wb_ref.at[:, cs], sem.at[12 + p])

    def o_copy(q, n):
        return pltpu.make_async_copy(os_scr.at[pl.ds(q, n)], o_ref.at[pl.ds(q, n)], o_sem.at[n % 4])

    woa_copy = pltpu.make_async_copy(woa_hbm, woa_ref, sem.at[15])
    wob_copy = [pltpu.make_async_copy(wob_hbm.at[:, 128 * j:128 * j + 128], wob_ref.at[j], sem.at[19 + j])
                for j in range(5)]
    gw_copy = pltpu.make_async_copy(gw_hbm, gw_ref, sem.at[17])

    def prep_blk(p, j):
        jj = j + 5 * (p % 2)
        w = wb_ref[128 * j:128 * j + 128, p * D:(p + 1) * D].astype(f32)
        wtf_scr[jj] = w.T
        for d in range(DH):
            r = (p * D + H * d) // 2
            wtp_scr[r:r + H // 2, 128 * j:128 * j + 128] = _pack16(wtf_scr[jj, pl.ds(d, H, stride=DH), :])

    def prep_wb(p):
        for j in range(5):
            prep_blk(p, j)

    def prep_wob():
        wu = wob_ref.bitcast(u32)
        for j in range(5):
            for e in range(DH // 2):
                w = wu[j, pl.ds(e, H, stride=DH // 2), :]
                lo = jnp.concatenate([w[0:8], w[16:24]], axis=0)
                hi = jnp.concatenate([w[8:16], w[24:32]], axis=0)
                wobp_scr[H * e:H * e + H // 2, 128 * j:128 * j + 128] = (lo & 0xFFFF) | (hi << 16)
                wobp_scr[H * e + H // 2:H * e + H, 128 * j:128 * j + 128] = (lo >> 16) | (hi & jnp.uint32(0xFFFF0000))

    def body(kind, step):
        first = kind == 0
        last = kind == 2
        if first:
            for i in range(3):
                x0_cols(i, 0).start()
                x0_cols(i, 1).start()
                if i == 0:
                    wa_cols(0).start()
                wa_cols(i + 1).start()
            wa_cols(4).start()
            wa_cols(5).start()
            gw_copy.start()
            for p in range(2):
                wb_copy(p).start()
            for c in wob_copy:
                c.start()
            woa_copy.start()
            x_copy.start()
            kb_scr[0, :, 0:HIST, :] = jnp.zeros((5, HIST, 128), f32)
            vb_scr[0, :, 0:HIST, :] = jnp.zeros((5, HIST, 128), f32)
            x_ref = x_scr.at[0]
        else:
            x_ref = x_scr.at[LAST if last else step]

        never = jax.lax.broadcasted_iota(jnp.int32, (BCH, 128), 0) + step < 0
        blk0 = 0 if first else NSB * LAST if last else NSB * step
        k_win = k_scr.at[pl.ds(blk0, 4)]
        vt_win = vt_scr.at[pl.ds(blk0, 4)]
        k_rd = [k_scr.at[pl.ds(blk0 + jnp.minimum(step, 0) * (i + 1), 4)] for i in range(NSB * GH)]

        def set_gate(sb, xs):
            if first:
                gw = gw_ref[...].reshape(1, D).astype(f32)
                gwf_scr[...] = jnp.broadcast_to(gw, (8, D))
            else:
                gw = gwf_scr[0:1, :]
            gate = jax.nn.sigmoid(jnp.sum(xs * gw, axis=1, keepdims=True))
            g_scr[sb * SUB:(sb + 1) * SUB, :] = jnp.broadcast_to(gate, (SUB, 128))

        if not first:
            set_gate(1, x_scr[LAST - 1 if last else step - 1, SUB:TQ, :].astype(f32))
        def xforms(x):
            xp = _bf(_pack16(x.astype(f32)))
            xu = pltpu.bitcast(x, u32)
            x_ev = pltpu.unpack_elementwise(xu, index=0, packed_dtype=bf16, unpacked_dtype=f32)
            x_od = pltpu.unpack_elementwise(xu, index=1, packed_dtype=bf16, unpacked_dtype=f32)
            xe = jnp.concatenate([t[8 * i:8 * i + 8] for i in range(x.shape[0] // 16) for t in (x_ev, x_od)],
                                 axis=0).astype(bf16)
            return x, xe, xp

        XS = []
        if last:
            XS.append(x_ref[...])
            set_gate(0, XS[0][0:SUB].astype(f32))
            set_gate(2, XS[0][SUB:TQ].astype(f32))
        elif not first:
            XS.extend(xforms(x_ref[...]))
            set_gate(0, XS[0][0:SUB].astype(f32))

        def pb(sb, n0, n1):
            rs = slice(sb * SUB, (sb + 1) * SUB)
            xr = (x_ref if first else XS[0])[min(sb, 1) * SUB:(min(sb, 1) + 1) * SUB]
            res = jax.lax.dot_general(xr, _bf(wtp_scr[64 * n0:64 * n1, :]), NT, preferred_element_type=f32)
            for n in range(n0, n1):
                p, c = divmod(n, 5)
                v = res[:, 128 * (n - n0):128 * (n - n0) + 128]
                if p == 0:
                    qb_scr[c, rs, :] = v * QSCALE
                else:
                    dst = kb_scr if p == 1 else vb_scr
                    dst[sb, c, HIST:HIST + SUB, :] = v
                    if sb < 2:
                        dst[2 if last else 1 - sb, c, 0:HIST, :] = v[SUB - HIST:SUB]
            return res

        def b_chunk(sb, ci, dep):
            r0 = ci * BCH
            R0 = sb * SUB + r0
            qb = [qb_scr[c, R0:R0 + BCH, :] for c in range(5)]
            if dep is not None:
                qb = [jnp.where(never, dep, q) for q in qb]
            logits = []
            for w in range(W_B):
                off = HIST - DIL * w + r0
                acc = qb[0] * kb_scr[sb, 0, off:off + BCH, :]
                for c in range(1, 5):
                    acc = acc + qb[c] * kb_scr[sb, c, off:off + BCH, :]
                acc = acc + pltpu.roll(acc, 64, 1)
                acc = acc + pltpu.roll(acc, 32, 1)
                if first and r0 < DIL * w:
                    pos = r0 + jax.lax.broadcasted_iota(jnp.int32, (BCH, 128), 0)
                    acc = jnp.where(pos >= DIL * w, acc, NEG)
                logits.append(acc)
            m = functools.reduce(jnp.maximum, logits)
            es = [jnp.exp2(l - m) for l in logits]
            den = functools.reduce(lambda a, b: a + b, es)
            fac = (1.0 - g_scr[R0:R0 + BCH, :]) / den
            for c in range(5):
                acc = None
                for w in range(W_B):
                    off = HIST - DIL * w + r0
                    term = es[w] * vb_scr[sb, c, off:off + BCH, :]
                    acc = term if acc is None else acc + term
                acc = acc * fac
                ob_scr[R0:R0 + BCH, 128 * c:128 * c + 128] = acc.astype(bf16)
            return acc

        deps = []

        def attn_b(sb, chain):
            for ci in range(SUB // BCH):
                deps.append(b_chunk(sb, ci, deps[-chain] if chain and len(deps) >= chain else None))

        written = [(q, 4) for q in range(0, S // 32 - 8, 4)]

        def emit(sb, v, init, fin):
            rs = slice(sb * SUB, (sb + 1) * SUB)
            if not init:
                v = acc_scr[rs, :] + v
            if fin:
                q0 = 0 if first else 8 * (LAST if last else step) + (0, -4, 4)[sb]
                os_scr[pl.ds(q0, 4)] = v.astype(bf16).reshape(4, 32, D)
                o_copy(q0, 4).start()
                if last and sb != 1:
                    written.append((q0, 4))
            else:
                acc_scr[rs, :] = v

        def op_b(sb, c0=0, c1=5, init=False, last=False, split=1):
            rs = slice(sb * SUB, (sb + 1) * SUB)
            n = SUB // split
            w = _bf(wobp_scr[64 * c0:64 * c1, :])
            v = jnp.concatenate([jnp.dot(ob_scr[sb * SUB + n * i:sb * SUB + n * i + n, 128 * c0:128 * c1], w,
                                         preferred_element_type=f32) for i in range(split)], axis=0)
            emit(sb, v, init, last)
            return v

        def op_a(sb, c0, c1, init=False, last=False, split=1):
            rs = slice(sb * SUB, (sb + 1) * SUB)
            gg = g_scr[rs, :]
            oa = ot_scr[128 * c0:128 * c1, min(sb, 1) * SUB:(min(sb, 1) + 1) * SUB].T
            oa = jnp.concatenate([oa[:, 128 * c:128 * c + 128] * gg for c in range(c1 - c0)], axis=1).astype(bf16)
            n = SUB // split
            w = woa_ref[128 * c0:128 * c1, :]
            v = jnp.concatenate([jnp.dot(oa[n * i:n * i + n], w, preferred_element_type=f32) for i in range(split)],
                                axis=0)
            emit(sb, v, init, last)
            return v

        def op_fin(sb, c0, c1, rows):
            gg = g_scr[sb * SUB:(sb + 1) * SUB, :]
            oa = ot_scr[128 * c0:128 * c1, min(sb, 1) * SUB:(min(sb, 1) + 1) * SUB].T
            oa = jnp.concatenate([oa[:, 128 * c:128 * c + 128] * gg for c in range(c1 - c0)], axis=1).astype(bf16)
            r = 0
            for n in rows:
                v = jnp.dot(oa[32 * r:32 * (r + n)], woa_ref[128 * c0:128 * c1, :], preferred_element_type=f32)
                v = v + acc_scr[sb * SUB + 32 * r:sb * SUB + 32 * (r + n), :]
                q0 = 8 * LAST + 2 * sb + r
                os_scr[pl.ds(q0, n)] = v.astype(bf16).reshape(n, 32, D)
                o_copy(q0, n).start()
                written.append((q0, n))
                r += n

        def dot_a(p):
            return jnp.dot(XS[p], wa_ref[:, p * D:(p + 1) * D], preferred_element_type=f32)

        def dot_k(k0, k1, lhs, c0, c1, split=1, r0=0, r1=2 * TQ):
            n = (r1 - r0) // split
            w = wa_ref[k0:k1, c0:c1]
            v = jnp.concatenate([jnp.dot(lhs[r0 + n * s:r0 + n * s + n], w, preferred_element_type=f32)
                                 for s in range(split)], axis=0)
            if k0 > 0:
                v = v + pa_scr[r0:r1, c0:c1]
            if k1 < D:
                pa_scr[r0:r1, c0:c1] = v
            return v

        def xs2(c0, c1):
            return xforms(jnp.concatenate([x_scr[0, :, c0:c1], x_scr[LAST, :, c0:c1]], axis=0))

        def post_v(va, far=0):
            vat = va.T
            rid = jax.lax.broadcasted_iota(jnp.int32, (VW, TQ), 0)
            for h in range(H):
                base, o, r = _vwin(h)
                win = jnp.where(rid == r, 1.0, vat[base:base + VW, :])
                for sb in range(NSB):
                    (vt_scr.at[pl.ds(NSB * LAST, 4)] if far else vt_win)[2 + sb, h] = win[:, sb * SUB:(sb + 1) * SUB]

        def post_k(ka, far=0):
            for g in range(NG):
                for sb in range(NSB):
                    (k_scr.at[pl.ds(NSB * LAST, 4)] if far else k_win)[2 + sb, g] = _pack16(ka[sb * SUB:(sb + 1) * SUB, G_OFF[g]:G_OFF[g] + 128])

        def post_q(qa, far=0):
            qp = pltpu.bitcast((qa * QSCALE).T.astype(bf16), u32)
            row8 = jax.lax.broadcasted_iota(jnp.int32, (8, 128), 0)
            for g in range(NG):
                for sb in range(NSB):
                    blk = qp[QR * g:QR * g + QR, sb * SUB:(sb + 1) * SUB]
                    r = [blk[0:16]] + [pltpu.roll(blk[8 * j:8 * j + 16], QB * j, 1) for j in range(1, GH)]
                    z = [r[0][0:8]]
                    for j in range(1, GH):
                        z.append(jnp.where(row8 < 2 * j, r[j - 1][8:16], r[j][0:8]))
                    z.append(r[GH - 1][8:16])
                    q_scr[far, g, :, sb * SUB:(sb + 1) * SUB] = jnp.concatenate(z, axis=0)

        lane = jax.lax.broadcasted_iota(jnp.int32, (QB, 128), 1)
        krow = jax.lax.broadcasted_iota(jnp.int32, (QB, 128), 0)
        old_valid = krow > (lane & (QB - 1))
        qrow = jax.lax.broadcasted_iota(jnp.int32, (QR, 128), 0)
        qhead = sum((qrow >= (DH // 2) * j).astype(jnp.int32) for j in range(1, GH))
        qcode = (jax.lax.broadcasted_iota(jnp.int32, (QR, 128), 1) // QB - qhead) & (GH - 1)

        def masks(rows):
            slot = jax.lax.broadcasted_iota(jnp.int32, (rows, 128), 1) // QB
            return slot, (slot == 0) | (slot == 2), slot < 2, (slot == 1) | (slot == 2)

        def masks_after(dep):
            slot = jax.lax.broadcasted_iota(jnp.int32, (8, 128), 1) // QB
            slot = jnp.where(never, pltpu.bitcast(dep, jnp.int32), slot)
            slot = jnp.concatenate([slot, slot], axis=0)
            return slot, (slot & 1) == 0, slot < 2, ((slot + 1) & 2) != 0

        mk16 = masks(QB // 2)
        mk1 = masks(1)

        def butterfly(X, mk):
            slot, m_even, m_01, m_12 = mk

            def sel(m, a, b):
                if a is None and b is None:
                    return None
                z = jnp.zeros_like(a if b is None else b)
                return jnp.where(m, z if a is None else a, z if b is None else b)

            live = [t for t in range(GH) if X[t] is not None]
            if len(live) == 1:
                t = live[0]
                return [sel(slot == (j + t) % GH, X[t], None) for j in range(GH)]
            a0 = sel(m_even, X[0], X[1])
            a1 = sel(m_even, X[1], X[0])
            b0 = sel(m_even, X[2], X[3])
            b1 = sel(m_even, X[3], X[2])
            return [sel(m_01, a0, b0), sel(m_12, a1, b1), sel(m_01, b0, a0), sel(m_12, b1, a1)]

        st8 = {}

        def segs_of(idx):
            sb = idx // NG
            return tuple(range(2 - sb, 3)) if first else (0, 1, 2)

        def qweights(idx, t, dep=None):
            sb, g = divmod(idx, NG)
            z = q_scr[int(last), g, :, sb * SUB:(sb + 1) * SUB]
            if dep is not None:
                z = jnp.concatenate([jnp.where(never, pltpu.bitcast(dep, u32), z[0:8]), z[8:]], axis=0)
            w = jnp.where(qcode == t, z, jnp.zeros_like(z))
            ro = QR * g - G_OFF[g] // 2
            parts = [jnp.zeros((ro, 128), u32), w, jnp.zeros((64 - QR - ro, 128), u32)]
            return _bf(jnp.concatenate([p for p in parts if p.shape[0]], axis=0))

        def seg_range(t, seg):
            return max(4 * seg - t, 0), min(4 * seg + 4 - t, NU)

        def soft(idx, t, seg, chunks):
            S_ = st8.setdefault(idx, {'P': [dict() for _ in range(GH)], 'm': {}, 'o': {}})
            u0, u1 = seg_range(t, seg)
            ss = {}
            for u in range(u0, u1):
                s = chunks[u]
                if u == 0:
                    s = jnp.where(old_valid, s, NEG)
                if u == NU - 1:
                    s = jnp.where(old_valid, NEG, s)
                ss[u] = s
            mx = functools.reduce(jnp.maximum,
                                  [ss[u][8 * i:8 * i + 8] for u in range(u0, u1) for i in range(QB // 8)])
            m = jnp.max(mx, axis=0, keepdims=True)
            S_['m'][(t, seg)] = m
            for u in range(u0, u1):
                S_['P'][t][u] = _pack16(jnp.exp2(ss[u] - m))

        def qk(idx, dq=(None,) * GH):
            sb, g = divmod(idx, NG)
            segs = segs_of(idx)
            chunks = []
            for t in range(GH):
                u0 = seg_range(t, segs[0])[0]
                r0 = (sb * SUB + QB * t) // 2
                ra, rb = r0 + u0 * QB // 2, r0 + NU * QB // 2
                pcs = []
                for b in range(4):
                    lo, hi = max(ra, 64 * b), min(rb, 64 * b + 64)
                    if lo < hi:
                        pcs.append((k_win if first else k_rd[GH * sb + t])[b, g, lo - 64 * b:hi - 64 * b, :])
                kk = _bf(jnp.concatenate(pcs, axis=0))
                st = jax.lax.dot_general(kk, qweights(idx, t, dq[t]), NN, preferred_element_type=f32)
                chunks.append({u: st[QB * (u - u0):QB * (u - u0) + QB] for u in range(u0, NU)})
            for seg in segs:
                for t in ((3, 2, 1, 0) if seg < 2 else (0, 1, 2, 3)):
                    soft(idx, t, seg, chunks[t])
            return chunks

        def pv(idx, after=None):
            sb, g = divmod(idx, NG)
            segs = segs_of(idx)
            S_ = st8.pop(idx)
            for seg in segs:
                outs = [[] for _ in range(GH)]
                mk = mk16 if after is None or after[seg] is None else masks_after(after[seg])
                for c in range(4 * seg, 4 * seg + 4):
                    X = [S_['P'][t].get(c - t) for t in range(GH)]
                    for j, v in enumerate(butterfly(X, mk)):
                        outs[j].append(v)
                for j in range(GH):
                    h = GH * g + j
                    pt = _bf(jnp.concatenate(outs[j], axis=0))
                    vt = vt_win[sb + seg, h]
                    S_['o'][(j, seg)] = jax.lax.dot_general(vt, pt, NN, preferred_element_type=f32)
            al = {}
            if len(segs) > 1:
                mf = [functools.reduce(jnp.maximum, [S_['m'][(t, seg)] for seg in segs]) for t in range(GH)]
                for seg in segs:
                    al[seg] = butterfly([jnp.exp2(S_['m'][(t, seg)] - mf[t]) for t in range(GH)], mk1)
            for j in range(GH):
                h = GH * g + j
                if len(segs) > 1:
                    ot = functools.reduce(lambda a, b: a + b, [S_['o'][(j, seg)] * al[seg][j] for seg in segs])
                else:
                    ot = S_['o'][(j, segs[0])]
                base, o, r = _vwin(h)
                inv = 1.0 / ot[r:r + 1, :]
                on = ot * inv
                if j:
                    on = pltpu.roll(on, 128 - QB * j, 1)
                ot_scr[DH * h:DH * h + DH, sb * SUB:(sb + 1) * SUB] = on[o:o + DH, :]
            return on[0:8]

        nidx = NSB * NG

        def pace(ch):
            return [None, ch[0][1][0:8], ch[0][3][0:8]]

        if first:
            x0_cols(0, 0).wait()
            x0_cols(0, 1).wait()
            wa_cols(0).wait()
            xs = xs2(0, 128)
            dot_k(0, 128, xs[0], 0, 512)
            dot_k(0, 128, xs[0], 512, D, 4)
            wa_cols(1).wait()
            dot_k(0, 128, xs[1], D, 2 * D)
            dot_k(0, 128, xs[2], 2 * D, 2 * D + 384)
            dot_k(0, 128, xs[2], 2 * D + 384, 3 * D, 2)
            x0_cols(1, 0).wait()
            x0_cols(1, 1).wait()
            wa_cols(2).wait()
            xs = xs2(128, 256)
            dot_k(128, 256, xs[0], 0, D)
            dot_k(128, 256, xs[1], D, 2 * D)
            dot_k(128, 256, xs[2], 2 * D, 2 * D + 256)
            dot_k(128, 256, xs[2], 2 * D + 256, 3 * D, 4)
            x0_cols(2, 0).wait()
            x0_cols(2, 1).wait()
            wa_cols(3).wait()
            wa_cols(4).wait()
            xs = xs2(256, D)
            post_v(dot_k(256, D, xs[2], 2 * D, 3 * D, 1, 0, TQ))
            post_v(dot_k(256, D, xs[2], 2 * D, 3 * D, 1, TQ, 2 * TQ), 1)
            dot_k(256, 384, xs[0][:, 0:128], 0, D)
            dot_k(256, 384, xs[1][:, 0:128], D + 256, 2 * D)
            dot_k(256, 384, xs[1][:, 0:128], D, D + 256, 1, 0, TQ)
            wa_cols(5).wait()
            wb_copy(0).wait()
            gw_copy.wait()
            xs = xforms(x_scr[0, :, 384:D])
            x7 = xforms(x_scr[LAST, :, 256:D])

            def far(p, k0, c0, c1, split=1):
                cs = slice(p * D + c0, p * D + c1)
                n = TQ // split
                v = jnp.concatenate([jnp.dot(x7[p][n * i:n * i + n, k0 - 256:], wa_ref[k0:D, cs], preferred_element_type=f32)
                                     for i in range(split)], axis=0) + pa_scr[TQ:2 * TQ, cs]
                pa_scr[TQ:2 * TQ, cs] = v
                return v

            post_q(dot_k(384, D, xs[0], 0, D, 1, 0, TQ))
            prep_wb(0)
            post_k(dot_k(384, D, xs[1], D, 2 * D, 1, 0, TQ))
            set_gate(0, x_ref[0:SUB].astype(f32))
            far(1, 256, 0, 256)
            far(1, 384, 256, 640)
            post_k(pa_scr[TQ:2 * TQ, D:2 * D], 1)
            seq = [i // 2 + NG * (1 - i % 2) for i in range(nidx)]
            for i in range(nidx):
                qk(seq[i])
                if i in (2, 4, 6, 8):
                    pb(0, i // 2 - 1, i // 2)
                if i >= 2:
                    pv(seq[i - 2])
            far(0, 384, 0, 256, 2)
            pv(15)
            far(0, 384, 256, 512, 2)
            pv(7)
            far(0, 384, 512, 640, 2)
            wb_copy(1).wait()
            for c in wob_copy:
                c.wait()
            woa_copy.wait()
            prep_wb(1)
            prep_wb(2)
            pb(0, 4, 5)
            pb(1, 0, 5)
            pb(0, 10, 15)
            pb(0, 5, 10)
            post_q(pa_scr[TQ:2 * TQ, 0:D], 1)
            attn_b(0, 4)
            pb(1, 5, 10)
            prep_wob()
            pb(1, 10, 15)
            op_a(0, 0, 5, init=True)
            op_b(0, last=True)
            x_copy.wait()
        elif last:
            attn_b(1, 3)
            pb(0, 0, 15)
            pb(2, 0, 15)
            attn_b(0, 3)
            op_a(1, 0, 5, init=True)
            op_b(1, last=True)
            attn_b(2, 3)
            fill = {8: (0, 3), 10: (3, 4), 11: (4, 5)}
            for idx in range(nidx):
                dp = pace(qk(idx, deps[-4:]) if idx == 3 else qk(idx))
                if idx > 0:
                    pv(idx - 1, dp)
                if idx in fill:
                    op_a(0, *fill[idx], init=idx == 8)
            op_b(0, last=True)
            op_b(2, init=True)
            pv(nidx - 1)
            op_a(2, 0, 3)
            op_fin(2, 3, 5, [1, 1, 1, 1])
            assert sum(n for _, n in written) == S // 32
            for q, n in written:
                o_copy(q, n).wait()
        else:
            attn_b(1, 2)
            post_v(dot_a(2))
            pb(0, 0, 15)
            attn_b(0, 2)
            post_k(dot_a(1))
            op_a(1, 0, 5, init=True)
            op_b(1, last=True)
            post_q(dot_a(0))
            op_b(0, init=True)
            fill = {2: (0, 3), 5: (3, 7), 9: (7, 11), 12: (11, 15)}
            for idx in range(nidx + 1):
                dp = [None, ra[0:8, 128:256], ra[0:8, 384:512]] if idx == nidx else None
                if idx < nidx:
                    dp = pace(qk(idx))
                if idx in fill:
                    r = pb(1, *fill[idx])
                    nn = fill[idx][1] - fill[idx][0]
                    dp = [(dp[s] if n is None or nn + n < 0 else r[ro:ro + 8, 128 * (nn + n):128 * (nn + n) + 128])
                          for s, (n, ro) in enumerate([(-4, 0), (-3, 64), (-2, 0)])]
                if idx > 0:
                    pv(idx - 1, dp)
                if idx == 15:
                    ra = op_a(0, 0, 4)
                if idx == 16:
                    op_a(0, 4, 5, last=True, split=4)

    @pl.when(pid == 0)
    def _():
        body(0, pid)

        @pl.loop(1, LAST)
        def _(i):
            body(1, i)

        body(2, pid)


@jax.jit
def pallas_gated_mix__sliding_block__sliding_local_dilated__prompt_kernel(A_x, A_wqkv, A_wo, B_x, B_wqkv, B_wo, gate_w):
    x = A_x.reshape(NSTEP, TQ, D)
    hbm = pl.BlockSpec(memory_space=pl.ANY)
    out = pl.pallas_call(
        _kernel,
        grid=(2,),
        in_specs=[hbm] * 6,
        out_specs=hbm,
        out_shape=jax.ShapeDtypeStruct((S // 32, 32, D), bf16),
        scratch_shapes=[
            pltpu.VMEM((NSTEP, TQ, D), bf16),
            pltpu.VMEM((D, 3 * D), bf16),
            pltpu.VMEM((D, D), bf16),
            pltpu.VMEM((D, 3 * D), bf16),
            pltpu.VMEM((5, D, 128), bf16),
            pltpu.VMEM((D,), bf16),
            pltpu.VMEM((S // SUB + 2, NG, SUB // 2, 128), u32),
            pltpu.VMEM((S // SUB + 2, H, VW, SUB), f32),
            pltpu.VMEM((2, NG, QR, TQ), u32),
            pltpu.VMEM((D, TQ), f32),
            pltpu.VMEM((10, D, 128), f32),
            pltpu.VMEM((3 * D // 2, D), u32),
            pltpu.VMEM((D // 2, D), u32),
            pltpu.VMEM((5, 3 * SUB, 128), f32),
            pltpu.VMEM((3, 5, HIST + SUB, 128), f32),
            pltpu.VMEM((3, 5, HIST + SUB, 128), f32),
            pltpu.VMEM((3 * SUB, D), bf16),
            pltpu.VMEM((3 * SUB, 128), f32),
            pltpu.VMEM((S // 32, 32, D), bf16),
            pltpu.SemaphoreType.DMA((4,)),
            pltpu.VMEM((3 * SUB, D), f32),
            pltpu.VMEM((2 * TQ, 3 * D), f32),
            pltpu.SemaphoreType.DMA((24,)),
            pltpu.VMEM((8, D), f32),
        ],
        compiler_params=pltpu.CompilerParams(
            dimension_semantics=("arbitrary",),
            vmem_limit_bytes=100 * 1024 * 1024,
            disable_bounds_checks=True,
            disable_semaphore_checks=True,
        ),
    )(x, A_wqkv, A_wo, B_wqkv, B_wo, gate_w)
    return out.reshape(1, S, D)
```
